```python
import jax
import jax.numpy as jnp

def _softmax(x, axis=-1):
    return jax.nn.softmax(x, axis=axis)
def _gelu(x):
    return jax.nn.gelu(x, approximate=True)
def _silu(x):
    return jax.nn.silu(x)
def _sigmoid(x):
    return jax.nn.sigmoid(x)
def _layernorm(x, axis=-1, eps=1e-5):
    m = jnp.mean(x, axis=axis, keepdims=True)
    v = jnp.var(x, axis=axis, keepdims=True)
    return (x - m) / jnp.sqrt(v + eps)
def _scatter_add(tgt, idx, src, axis=0):
    return tgt.at[idx].add(src)
def _segment_sum(src, seg, n):
    return jax.ops.segment_sum(src, seg, n)
class _Rng:
    def __init__(self, key):
        self._k = key
    def _next(self):
        self._k, sub = jax.random.split(self._k)
        return sub
    def normal(self, shape):
        return jax.random.normal(self._next(), shape, dtype=jnp.bfloat16)
    def randint(self, lo, hi, shape):
        return jax.random.randint(self._next(), shape, lo, hi, dtype=jnp.int32)
    def uniform(self, shape, lo=0.0, hi=1.0):
        return jax.random.uniform(self._next(), shape, jnp.bfloat16, lo, hi)
    def permutation(self, n):
        return jax.random.permutation(self._next(), n)


kernel_name = 'parallel_sum__ssm_conv_s5__moe_arch_mod__prompt'

def setup_inputs():
    _rng = _Rng(jax.random.key(int.from_bytes(__import__("os").urandom(4), "little")))
    _w = (lambda a: (lambda t: t.astype(jnp.bfloat16) if jnp.issubdtype(t.dtype, jnp.floating) else t)(jnp.asarray(a)))
    def _A_setup():
        B, S, D = 1, 2048, 1024
        P = D
        Lambda_re = -0.5 * jnp.exp((lambda *s: _rng.normal(s) * 0.05)(P))
        Lambda_im = (lambda *s: _rng.normal(s) * 0.05)(P) * 1.0
        B_re = (lambda *s: _rng.normal(s) * 0.05)(P, D) * (D ** -0.5)
        B_im = (lambda *s: _rng.normal(s) * 0.05)(P, D) * (D ** -0.5)
        C_re = (lambda *s: _rng.normal(s) * 0.05)(D, P) * (P ** -0.5)
        C_im = (lambda *s: _rng.normal(s) * 0.05)(D, P) * (P ** -0.5)
        log_dt = (lambda *s: _rng.normal(s) * 0.05)(P) * 0.3 - 2.0
        Dskip = (lambda *s: _rng.normal(s) * 0.05)(D)
        return {
            "x": _w((lambda *s: _rng.normal(s) * 0.05)(B, S, D)),
            "Lambda_re": _w(Lambda_re),
            "Lambda_im": _w(Lambda_im),
            "B_re": _w(B_re),
            "B_im": _w(B_im),
            "C_re": _w(C_re),
            "C_im": _w(C_im),
            "log_dt": _w(log_dt),
            "Dskip": _w(Dskip),
        }
    _A_in = _A_setup()

    def _B_setup():
        B, S, D, F, C = 1, 2048, 1024, 3584, 2
        return {
            "x": _w((lambda *s: _rng.normal(s) * 0.05)(B, S, D)),
            "w_r": _w((lambda *s: _rng.normal(s) * 0.05)(D)),
            "w_gate": _w((lambda *s: _rng.normal(s) * 0.05)(D, F)),
            "w_up": _w((lambda *s: _rng.normal(s) * 0.05)(D, F)),
            "w_down": _w((lambda *s: _rng.normal(s) * 0.05)(F, D)),
        }
    _B_in = _B_setup()

    return {
        "A_x": _A_in["x"],
        "A_Lambda_re": _A_in["Lambda_re"],
        "A_Lambda_im": _A_in["Lambda_im"],
        "A_B_re": _A_in["B_re"],
        "A_B_im": _A_in["B_im"],
        "A_C_re": _A_in["C_re"],
        "A_C_im": _A_in["C_im"],
        "A_log_dt": _A_in["log_dt"],
        "A_Dskip": _A_in["Dskip"],
        "B_x": _B_in["x"],
        "B_w_r": _B_in["w_r"],
        "B_w_gate": _B_in["w_gate"],
        "B_w_up": _B_in["w_up"],
        "B_w_down": _B_in["w_down"],
    }

def reference(A_x, A_Lambda_re, A_Lambda_im, A_B_re, A_B_im, A_C_re, A_C_im, A_log_dt, A_Dskip, B_x, B_w_r, B_w_gate, B_w_up, B_w_down):
    def _A_ref(x, Lambda_re, Lambda_im, B_re, B_im, C_re, C_im, log_dt, Dskip):
        Bsz, L, H = x.shape
        Lam = Lambda_re + 1j * Lambda_im
        Bmat = B_re + 1j * B_im
        Cmat = C_re + 1j * C_im
        dt = jnp.exp(log_dt)
        Lam_bar = jnp.exp(dt * Lam)
        B_bar = ((Lam_bar - 1.0) / Lam)[:, None] * Bmat
        Bu = jnp.einsum("bld,pd->blp", x + 0j, B_bar)
        h = jnp.zeros_like(Bu[:, 0, :])
        hs = []
        for t in range(L):
            h = Lam_bar[None, :] * h + Bu[:, t, :]
            hs.append(h)
        hseq = jnp.stack(hs, 1)
        y = 2.0 * jnp.einsum("blp,dp->bld", hseq, Cmat).real + x * Dskip[None, None, :]
        return y

    def _B_ref(x, w_r, w_gate, w_up, w_down):
        B, S, D = x.shape
        C = 2
        r = x @ w_r
        idx = jnp.argsort(-r, axis=-1)[:, :C]
        idx_e = jnp.repeat(idx.reshape(B, C, 1), D, axis=2)
        x_sel = jnp.take_along_axis(x, idx_e, axis=1)
        g = _silu(x_sel @ w_gate)
        u = x_sel @ w_up
        y = (g * u) @ w_down
        r_sel = _sigmoid(jnp.take_along_axis(r, idx, axis=1))
        y = y * r_sel.reshape(B, C, 1)
        b_off = (jnp.arange(B) * S).reshape(B, 1)
        flat_idx = (idx + b_off).reshape(B * C)
        zero = (x * 0.0).reshape(B * S, D)
        upd = _scatter_add(zero, flat_idx, y.reshape(B * C, D), axis=0)
        return x + upd.reshape(B, S, D)

    x = A_x
    xn = _layernorm(x, axis=-1)
    return x + _A_ref(xn, A_Lambda_re, A_Lambda_im, A_B_re, A_B_im, A_C_re, A_C_im, A_log_dt, A_Dskip) + _B_ref(xn, B_w_r, B_w_gate, B_w_up, B_w_down)
```

```python
import jax
import jax.numpy as jnp
import numpy as np
import jax.experimental.pallas as pl
import jax.experimental.pallas.tpu as pltpu

L = 2048
D = 1024
P = 1024
F = 3584
NSEG = 8
SEG = L // NSEG
J = 32
NB = SEG // J
R = NSEG * J
G = D // 128

_NT = (((1,), (1,)), ((), ()))
f32 = jnp.float32
bf16 = jnp.bfloat16


def _rb(v):
    return v.astype(bf16).astype(f32)


def _kernel(x_hbm, lre_ref, lim_ref, bre_hbm, bim_hbm, cre_hbm, cim_hbm, ldt_ref,
            dsk_ref, wr_ref, wg_hbm, wu_hbm, wd_hbm, out_hbm,
            x_v, xn_v, b_v, craw_v, c_v, bu_v, h_v, o_v, st_v, wg_v, wu_v, wd_v,
            sx, sw, so):
    def x_cp(b, s):
        rows = pl.ds(s * SEG, J) if b == 0 else pl.ds(s * SEG + J, SEG - J)
        return [pltpu.make_async_copy(x_hbm.at[rows], x_v.at[rows], sx.at[b])]

    def o_cp(b, s):
        rows = pl.ds(pl.multiple_of(s * SEG + b * J, J), J)
        return pltpu.make_async_copy(o_v.at[rows], out_hbm.at[rows], so.at[0])

    b_cps = [pltpu.make_async_copy(bre_hbm, b_v.at[pl.ds(0, P)], sw.at[0]),
             pltpu.make_async_copy(bim_hbm, b_v.at[pl.ds(P, P)], sw.at[1])]
    c_cps = [pltpu.make_async_copy(cre_hbm, craw_v.at[0], sw.at[2]),
             pltpu.make_async_copy(cim_hbm, craw_v.at[1], sw.at[3])]
    f_cps = [pltpu.make_async_copy(wg_hbm, wg_v, sw.at[4]),
             pltpu.make_async_copy(wu_hbm, wu_v, sw.at[5]),
             pltpu.make_async_copy(wd_hbm, wd_v, sw.at[6])]

    for s in range(NSEG):
        for c in x_cp(0, s):
            c.start()
    for c in b_cps:
        c.start()

    dt = _rb(jnp.exp(ldt_ref[...].astype(f32)))
    lre = lre_ref[...].astype(f32)
    lim = lim_ref[...].astype(f32)
    mag = jnp.exp(dt * lre)
    a_re = mag * jnp.cos(dt * lim)
    a_im = mag * jnp.sin(dt * lim)
    den = lre * lre + lim * lim
    k_re = 2.0 * ((a_re - 1.0) * lre + a_im * lim) / den
    k_im = 2.0 * (a_im * lre - (a_re - 1.0) * lim) / den
    ar8 = jnp.broadcast_to(a_re, (NSEG, P))
    ai8 = jnp.broadcast_to(a_im, (NSEG, P))
    wr = wr_ref[...].astype(f32)
    eps = f32(np.float32(np.asarray(1e-5, dtype=bf16)))

    dsk = dsk_ref[...].astype(f32)
    lane = jax.lax.broadcasted_iota(jnp.int32, (NSEG, SEG), 1)
    sub = jax.lax.broadcasted_iota(jnp.int32, (NSEG, SEG), 0)

    def phase_a(b, carry, first=False):
        hr, hi, racc = carry
        if first:
            for s in range(NSEG):
                for c in x_cp(0, s):
                    c.wait()
        rows = pl.ds(pl.multiple_of(b * R, R), R)
        for s in range(NSEG):
            nat = pl.ds(pl.multiple_of(s * SEG + b * J, J), J)
            x = x_v[nat, :].astype(f32)
            m = jnp.sum(x, axis=-1, keepdims=True) * (1.0 / D)
            c = x - m
            v = jnp.sum(c * c, axis=-1, keepdims=True) * (1.0 / D)
            sd = _rb(jnp.sqrt(_rb(_rb(v) + eps)))
            xn = _rb(_rb(x - _rb(m)) / sd)
            o_v[nat, :] = x + _rb(xn * dsk) + xn
            for g in range(G):
                st_v[g, pl.ds(s, J, stride=NSEG), :] = xn[:, 128 * g:128 * (g + 1)]
        xn = jnp.concatenate([st_v[g] for g in range(G)], axis=1)
        r = _rb(jnp.sum(xn * wr, axis=-1, keepdims=True))
        xn = xn.astype(bf16)
        xn_v[rows, :] = xn
        for j in range(J):
            racc = jnp.where(lane == b * J + j, r[NSEG * j:NSEG * (j + 1), :], racc)
        if first:
            for cp in b_cps:
                cp.wait()
            for s in range(NSEG):
                for c in x_cp(1, s):
                    c.start()
            for cp in c_cps + f_cps:
                cp.start()
        bu = jax.lax.dot_general(xn, b_v[...], _NT, preferred_element_type=f32)
        bu_v[rows, :] = bu
        for j in range(J):
            br = bu[NSEG * j:NSEG * (j + 1), :P]
            bi = bu[NSEG * j:NSEG * (j + 1), P:]
            hr, hi = ar8 * hr - ai8 * hi + br, ar8 * hi + ai8 * hr + bi
        return hr, hi, racc

    z = jnp.zeros((NSEG, P), f32)
    carry = phase_a(0, (z, z, jnp.zeros((NSEG, SEG), f32)), first=True)
    for s in range(NSEG):
        for c in x_cp(1, s):
            c.wait()
    er, ei, racc = jax.lax.fori_loop(1, NB, phase_a, carry)

    pr, pi = ar8, ai8
    n = 1
    while n < SEG:
        pr, pi = pr * pr - pi * pi, 2.0 * pr * pi
        n *= 2
    srow = jax.lax.broadcasted_iota(jnp.int32, (NSEG, P), 0)
    hr = jnp.where(srow >= 1, pltpu.roll(er, 1, 0), 0.0)
    hi = jnp.where(srow >= 1, pltpu.roll(ei, 1, 0), 0.0)
    for sh in (1, 2, 4):
        tr = jnp.where(srow >= sh, pltpu.roll(hr, sh, 0), 0.0)
        ti = jnp.where(srow >= sh, pltpu.roll(hi, sh, 0), 0.0)
        hr, hi = hr + pr * tr - pi * ti, hi + pr * ti + pi * tr
        pr, pi = pr * pr - pi * pi, 2.0 * pr * pi

    for cp in c_cps:
        cp.wait()
    cre = craw_v[0].astype(f32)
    cim = craw_v[1].astype(f32)
    c_v[:, :P] = (cre * k_re - cim * k_im).astype(bf16)
    c_v[:, P:] = (-(cre * k_im + cim * k_re)).astype(bf16)

    tok = sub * SEG + lane
    r0 = jnp.max(racc)
    i0 = jnp.min(jnp.where(racc == r0, tok, L))
    rest = jnp.where(tok == i0, -jnp.inf, racc)
    r1 = jnp.max(rest)
    i1 = jnp.min(jnp.where((rest == r1) & (tok != i0), tok, L))
    i0 = jnp.clip(i0, 0, L - 1)
    i1 = jnp.clip(i1, 0, L - 1)
    p0 = (i0 % SEG) * NSEG + i0 // SEG
    p1 = (i1 % SEG) * NSEG + i1 // SEG
    r16 = jax.lax.broadcasted_iota(jnp.int32, (16, D), 0)

    def pick(p):
        g = xn_v[pl.ds(pl.multiple_of((p // 16) * 16, 16), 16), :].astype(f32)
        return jnp.sum(jnp.where(r16 == p % 16, g, 0.0), axis=0, keepdims=True)

    xs = jnp.where(r16 == 0, pick(p0), jnp.where(r16 == 1, pick(p1), 0.0)).astype(bf16)
    for cp in f_cps:
        cp.wait()
    g = _rb(jnp.dot(xs, wg_v[...], preferred_element_type=f32))
    u = _rb(jnp.dot(xs, wu_v[...], preferred_element_type=f32))
    g = _rb(g * jax.nn.sigmoid(g))
    y = _rb(jnp.dot((g * u).astype(bf16), wd_v[...], preferred_element_type=f32))
    rs = jnp.where(r16 == 0, r0, r1)
    y = _rb(y * _rb(jax.nn.sigmoid(rs)))
    y0 = y[0:1, :]
    y1 = y[1:2, :]
    rowi = jax.lax.broadcasted_iota(jnp.int32, (R, D), 0)

    def phase_b(b, carry):
        hr, hi = carry
        base = pl.multiple_of(b * R, R)
        for jp in range(J // 2):
            rs_, is_ = [], []
            for j in (2 * jp, 2 * jp + 1):
                rows = pl.ds(base + NSEG * j, NSEG)
                br = bu_v[rows, :P]
                bi = bu_v[rows, P:]
                hr, hi = ar8 * hr - ai8 * hi + br, ar8 * hi + ai8 * hr + bi
                rs_.append(hr)
                is_.append(hi)
            h_v[16 * jp:16 * (jp + 1), :P] = jnp.concatenate(rs_, axis=0).astype(bf16)
            h_v[16 * jp:16 * (jp + 1), P:] = jnp.concatenate(is_, axis=0).astype(bf16)
        ys = jax.lax.dot_general(h_v[...], c_v[...], _NT, preferred_element_type=f32)
        ys = ys + jnp.where(rowi == p0 - base, y0, 0.0) + jnp.where(rowi == p1 - base, y1, 0.0)
        for g in range(G):
            st_v[g] = ys[:, 128 * g:128 * (g + 1)]
        for s in range(NSEG):
            nat = pl.ds(pl.multiple_of(s * SEG + b * J, J), J)
            o_v[nat, :] += jnp.concatenate(
                [st_v[g, pl.ds(s, J, stride=NSEG), :] for g in range(G)], axis=1)
        for s in range(NSEG):
            o_cp(b, s).start()
        return hr, hi

    jax.lax.fori_loop(0, NB, phase_b, (hr, hi))
    pltpu.make_async_copy(o_v, o_v, so.at[0]).wait()


@jax.jit
def pallas_parallel_sum__ssm_conv_s5__moe_arch_mod__prompt_kernel(
    A_x: jax.Array,
    A_Lambda_re: jax.Array,
    A_Lambda_im: jax.Array,
    A_B_re: jax.Array,
    A_B_im: jax.Array,
    A_C_re: jax.Array,
    A_C_im: jax.Array,
    A_log_dt: jax.Array,
    A_Dskip: jax.Array,
    B_x: jax.Array,
    B_w_r: jax.Array,
    B_w_gate: jax.Array,
    B_w_up: jax.Array,
    B_w_down: jax.Array,
):
    del B_x
    hbm = pl.BlockSpec(memory_space=pl.ANY)
    vec = pl.BlockSpec(memory_space=pltpu.VMEM)
    out = pl.pallas_call(
        _kernel,
        out_shape=jax.ShapeDtypeStruct((L, D), f32),
        in_specs=[hbm, vec, vec, hbm, hbm, hbm, hbm, vec, vec, vec, hbm, hbm, hbm],
        out_specs=hbm,
        scratch_shapes=[
            pltpu.VMEM((L, D), bf16),
            pltpu.VMEM((L, D), bf16),
            pltpu.VMEM((2 * P, D), bf16),
            pltpu.VMEM((2, D, P), bf16),
            pltpu.VMEM((D, 2 * P), bf16),
            pltpu.VMEM((L, 2 * P), f32),
            pltpu.VMEM((R, 2 * P), bf16),
            pltpu.VMEM((L, D), f32),
            pltpu.VMEM((G, R, 128), f32),
            pltpu.VMEM((D, F), bf16),
            pltpu.VMEM((D, F), bf16),
            pltpu.VMEM((F, D), bf16),
            pltpu.SemaphoreType.DMA((2,)),
            pltpu.SemaphoreType.DMA((7,)),
            pltpu.SemaphoreType.DMA((1,)),
        ],
        compiler_params=pltpu.CompilerParams(vmem_limit_bytes=100 * 1024 * 1024),
    )(
        A_x.reshape(L, D),
        A_Lambda_re.reshape(1, P), A_Lambda_im.reshape(1, P),
        A_B_re, A_B_im, A_C_re, A_C_im,
        A_log_dt.reshape(1, P), A_Dskip.reshape(1, D), B_w_r.reshape(1, D),
        B_w_gate, B_w_up, B_w_down,
    )
    return out.reshape(1, L, D)
```

```python
import jax
import jax.numpy as jnp
import numpy as np
import jax.experimental.pallas as pl
import jax.experimental.pallas.tpu as pltpu

L = 2048
D = 1024
P = 1024
F = 3584
NSEG = 8
SEG = L // NSEG
J = 32
NB = SEG // J
R = NSEG * J
G = D // 128
NA = 4
AHEAD = 3
PA = J + 4
PB = 12
NC = 2

_NT = (((1,), (1,)), ((), ()))
f32 = jnp.float32
bf16 = jnp.bfloat16


def _rb(v):
    return v.astype(bf16).astype(f32)


_cur=[None]
def _sc(n):
    if _cur[0] is not None: _cur[0].__exit__(None,None,None)
    _cur[0]=None
    if n:
        _cur[0]=jax.named_scope(n); _cur[0].__enter__()

def _kernel(x_hbm, lre_ref, lim_ref, bre_hbm, bim_hbm, cre_hbm, cim_hbm, ldt_ref,
            dsk_ref, wr_ref, wg_hbm, wu_hbm, wd_hbm, out_hbm,
            x_v, xn_v, b_v, craw_v, bu_v, h0_v, h1_v, o_v, st_v, wg_v, wu_v, wd_v,
            sx, sb, sw, so):
    def x_cp(b, s):
        rows = pl.ds(pl.multiple_of(s * SEG + b * J, J), J)
        return pltpu.make_async_copy(x_hbm.at[rows], x_v.at[rows], sx.at[b])

    def b_cp(n):
        w = 2 * P // NA
        src = bre_hbm if n < NA // 2 else bim_hbm
        return pltpu.make_async_copy(src.at[pl.ds(n * w % P, w)], b_v.at[pl.ds(n * w, w)], sb.at[n])

    def o_cp(b, s):
        rows = pl.ds(pl.multiple_of(s * SEG + b * J, J), J)
        return pltpu.make_async_copy(o_v.at[rows], out_hbm.at[rows], so.at[0])

    c_cps = [pltpu.make_async_copy(cre_hbm, craw_v.at[0], sw.at[2]),
             pltpu.make_async_copy(cim_hbm, craw_v.at[1], sw.at[3])]
    f_cps = [pltpu.make_async_copy(wg_hbm, wg_v, sw.at[4]),
             pltpu.make_async_copy(wu_hbm, wu_v, sw.at[5]),
             pltpu.make_async_copy(wd_hbm, wd_v, sw.at[6])]

    for b in range(AHEAD):
        for s in range(NSEG):
            x_cp(b, s).start()

    dt = _rb(jnp.exp(ldt_ref[...].astype(f32)))
    lre = lre_ref[...].astype(f32)
    lim = lim_ref[...].astype(f32)
    mag = jnp.exp(dt * lre)
    a_re = mag * jnp.cos(dt * lim)
    a_im = mag * jnp.sin(dt * lim)
    den = lre * lre + lim * lim
    k_re = 2.0 * ((a_re - 1.0) * lre + a_im * lim) / den
    k_im = 2.0 * (a_im * lre - (a_re - 1.0) * lim) / den
    ar8 = jnp.broadcast_to(a_re, (NSEG, P))
    ai8 = jnp.broadcast_to(a_im, (NSEG, P))
    wr = wr_ref[...].astype(f32)
    eps = f32(np.float32(np.asarray(1e-5, dtype=bf16)))

    dsk1 = dsk_ref[...].astype(f32) + 1.0
    lane = jax.lax.broadcasted_iota(jnp.int32, (NSEG, SEG), 1)
    sub = jax.lax.broadcasted_iota(jnp.int32, (NSEG, SEG), 0)

    def norm_rows(b, q, racc):
        x = jnp.concatenate([
            jnp.concatenate([st_v[g, pl.ds(2 * q + j, NSEG, stride=PA), :] for g in range(G)], axis=1)
            for j in range(2)], axis=0)
        m = jnp.sum(x, axis=-1, keepdims=True) * (1.0 / D)
        c = x - m
        v = jnp.sum(c * c, axis=-1, keepdims=True) * (1.0 / D)
        sd = _rb(jnp.sqrt(_rb(_rb(v) + eps)))
        xn = (_rb(x - _rb(m)) * (1.0 / sd)).astype(bf16)
        xn_v[pl.ds(pl.multiple_of(b * R + 16 * q, 16), 16), :] = xn
        r = _rb(jnp.sum(xn.astype(f32) * wr, axis=-1, keepdims=True))
        for j in range(2):
            racc = jnp.where(lane == b * J + 2 * q + j, r[NSEG * j:NSEG * (j + 1), :], racc)
        return racc

    def norm(b, racc):
        for s in range(NSEG):
            x_cp(b, s).wait()

        @pl.when(b + AHEAD < NB)
        def _():
            for s in range(NSEG):
                x_cp(b + AHEAD, s).start()

        for n in range(AHEAD):
            @pl.when(b + AHEAD == NB + n)
            def _():
                b_cp(n).start()

        for s in range(NSEG):
            nat = pl.ds(pl.multiple_of(s * SEG + b * J, J), J)
            for g in range(G):
                st_v[g, s * PA:s * PA + J, :] = x_v[nat, 128 * g:128 * (g + 1)].astype(f32)
        for q in range(R // 16):
            racc = norm_rows(b, q, racc)
        return racc

    def in_proj(b, n):
        rows = pl.ds(pl.multiple_of(b * R, R), R)
        cols = slice(n * 2 * P // NA, (n + 1) * 2 * P // NA)
        bu_v[rows, cols] = jax.lax.dot_general(
            xn_v[rows, :], b_v[cols, :], _NT, preferred_element_type=f32)

    def pass1(b, hr, hi, n=None):
        for j in range(J) if n is None else range(n * J // NA, (n + 1) * J // NA):
            rows = pl.ds(pl.multiple_of(b * R + NSEG * j, NSEG), NSEG)
            br = bu_v[rows, :P]
            bi = bu_v[rows, P:]
            hr, hi = ar8 * hr - ai8 * hi + br, ar8 * hi + ai8 * hr + bi
        return hr, hi

    def cprep(row):
        rows = pl.ds(pl.multiple_of(row, 16), 16)
        cre = craw_v[0, rows, :].astype(f32)
        cim = craw_v[1, rows, :].astype(f32)
        xn_v[pl.ds(pl.multiple_of(L + row, 16), 16), :] = (cre * k_re - cim * k_im).astype(bf16)
        xn_v[pl.ds(pl.multiple_of(L + D + row, 16), 16), :] = (cre * (-k_im) - cim * k_re).astype(bf16)

    z = jnp.zeros((NSEG, P), f32)
    _sc('a0')
    racc = jax.lax.fori_loop(0, NB, norm, jnp.zeros((NSEG, SEG), f32))
    _sc('a1')
    for n in range(NA):
        b_cp(n).wait()
        if n + AHEAD < NA:
            b_cp(n + AHEAD).start()
        if n + AHEAD == NA:
            for cp in c_cps + f_cps:
                cp.start()
        in_proj(0, n)
    _sc('aloop')

    def phase_a(b, carry, with_c=False):
        hr, hi, racc = carry
        for n in range(NA):
            in_proj(b, n)
            hr, hi = pass1(b - 1, hr, hi, n)
            if with_c:
                k = 2 * D // NB // NA
                for i in range(k // 16):
                    cprep(((b - NB // 2) * NA + n) * k + 16 * i)
        return hr, hi, racc

    hr, hi, racc = jax.lax.fori_loop(1, NB // 2, phase_a, (z, z, racc))
    for cp in c_cps:
        cp.wait()
    hr, hi, racc = jax.lax.fori_loop(
        NB // 2, NB, lambda b, c: phase_a(b, c, True), (hr, hi, racc))
    _sc('aend')
    er, ei = pass1(NB - 1, hr, hi)
    _sc('carry')
    pr, pi = ar8, ai8
    n = 1
    while n < SEG:
        pr, pi = pr * pr - pi * pi, 2.0 * pr * pi
        n *= 2
    srow = jax.lax.broadcasted_iota(jnp.int32, (NSEG, P), 0)
    hr = jnp.where(srow >= 1, pltpu.roll(er, 1, 0), 0.0)
    hi = jnp.where(srow >= 1, pltpu.roll(ei, 1, 0), 0.0)
    for sh in (1, 2, 4):
        tr = jnp.where(srow >= sh, pltpu.roll(hr, sh, 0), 0.0)
        ti = jnp.where(srow >= sh, pltpu.roll(hi, sh, 0), 0.0)
        hr, hi = hr + pr * tr - pi * ti, hi + pr * ti + pi * tr
        pr, pi = pr * pr - pi * pi, 2.0 * pr * pi

    _sc('top')
    tok = sub * SEG + lane
    r0 = jnp.max(racc)
    i0 = jnp.min(jnp.where(racc == r0, tok, L))
    rest = jnp.where(tok == i0, -jnp.inf, racc)
    r1 = jnp.max(rest)
    i1 = jnp.min(jnp.where((rest == r1) & (tok != i0), tok, L))
    i0 = jnp.clip(i0, 0, L - 1)
    i1 = jnp.clip(i1, 0, L - 1)
    p0 = (i0 % SEG) * NSEG + i0 // SEG
    p1 = (i1 % SEG) * NSEG + i1 // SEG
    r16 = jax.lax.broadcasted_iota(jnp.int32, (16, D), 0)

    def pick(p):
        g = xn_v[pl.ds(pl.multiple_of((p // 16) * 16, 16), 16), :].astype(f32)
        return jnp.sum(jnp.where(r16 == p % 16, g, 0.0), axis=0, keepdims=True)

    xs = jnp.where(r16 == 0, pick(p0), jnp.where(r16 == 1, pick(p1), 0.0)).astype(bf16)
    _sc('ffn')
    for cp in f_cps:
        cp.wait()
    g = _rb(jnp.dot(xs, wg_v[...], preferred_element_type=f32))
    u = _rb(jnp.dot(xs, wu_v[...], preferred_element_type=f32))
    g = _rb(g * jax.nn.sigmoid(g))
    y = _rb(jnp.dot((g * u).astype(bf16), wd_v[...], preferred_element_type=f32))
    rs = jnp.where(r16 == 0, r0, r1)
    y = _rb(y * _rb(jax.nn.sigmoid(rs)))
    y0 = y[0:1, :]
    y1 = y[1:2, :]
    rowt = jax.lax.broadcasted_iota(jnp.int32, (16, 128), 0)

    def pass2(b, h_v, hr, hi, n=None):
        base = pl.multiple_of(b * R, R)
        for jp in range(J // 2) if n is None else range(n * J // 2 // NC, (n + 1) * J // 2 // NC):
            rs_, is_ = [], []
            for j in (2 * jp, 2 * jp + 1):
                rows = pl.ds(base + NSEG * j, NSEG)
                br = bu_v[rows, :P]
                bi = bu_v[rows, P:]
                hr, hi = ar8 * hr - ai8 * hi + br, ar8 * hi + ai8 * hr + bi
                rs_.append(hr)
                is_.append(hi)
            h_v[16 * jp:16 * (jp + 1), :P] = jnp.concatenate(rs_, axis=0).astype(bf16)
            h_v[16 * jp:16 * (jp + 1), P:] = jnp.concatenate(is_, axis=0).astype(bf16)
        return hr, hi

    def out_proj(b, h_v, hn_v, hr, hi):
        w = D // NC
        for n in range(NC):
            cols = slice(n * w, (n + 1) * w)
            ys = jax.lax.dot_general(h_v[...], jnp.concatenate([xn_v[L + n * w:L + (n + 1) * w, :],
                                       xn_v[L + D + n * w:L + D + (n + 1) * w, :]], axis=1), _NT, preferred_element_type=f32)
            if hn_v is not None:
                hr, hi = pass2(b + 1, hn_v, hr, hi, n)
            for g in range(w // 128):
                gg = n * w // 128 + g
                cg = slice(128 * gg, 128 * (gg + 1))
                for q in range(R // 16):
                    row = pl.multiple_of(b * R + 16 * q, 16)
                    t = ys[16 * q:16 * (q + 1), 128 * g:128 * (g + 1)]
                    t = t + xn_v[pl.ds(row, 16), cg].astype(f32) * dsk1[:, cg]
                    t = jnp.where(rowt == p0 - row, t + y0[:, cg], t)
                    t = jnp.where(rowt == p1 - row, t + y1[:, cg], t)
                    for j in range(2):
                        st_v[gg, pl.ds(PB * (2 * q + j), 8), :] = t[8 * j:8 * (j + 1), :]
                for s in range(NSEG):
                    nat = pl.ds(pl.multiple_of(s * SEG + b * J, J), J)
                    o_v[nat, cg] = x_v[nat, cg].astype(f32) + st_v[gg, pl.ds(s, J, stride=PB), :]
        for s in range(NSEG):
            o_cp(b, s).start()
        return hr, hi

    _sc('b0')
    hr, hi = pass2(0, h0_v, hr, hi)
    _sc('bloop')

    def phase_b(i, carry):
        hr, hi = carry
        hr, hi = out_proj(2 * i, h0_v, h1_v, hr, hi)
        hr, hi = out_proj(2 * i + 1, h1_v, h0_v, hr, hi)
        return hr, hi

    hr, hi = jax.lax.fori_loop(0, NB // 2 - 1, phase_b, (hr, hi))
    _sc('bend')
    out_proj(NB - 2, h0_v, h1_v, hr, hi)
    out_proj(NB - 1, h1_v, None, hr, hi)
    _sc('tail')
    pltpu.make_async_copy(o_v, o_v, so.at[0]).wait()
    _sc(None)


@jax.jit
def pallas_parallel_sum__ssm_conv_s5__moe_arch_mod__prompt_kernel(
    A_x: jax.Array,
    A_Lambda_re: jax.Array,
    A_Lambda_im: jax.Array,
    A_B_re: jax.Array,
    A_B_im: jax.Array,
    A_C_re: jax.Array,
    A_C_im: jax.Array,
    A_log_dt: jax.Array,
    A_Dskip: jax.Array,
    B_x: jax.Array,
    B_w_r: jax.Array,
    B_w_gate: jax.Array,
    B_w_up: jax.Array,
    B_w_down: jax.Array,
):
    del B_x
    hbm = pl.BlockSpec(memory_space=pl.ANY)
    vec = pl.BlockSpec(memory_space=pltpu.VMEM)
    out = pl.pallas_call(
        _kernel,
        out_shape=jax.ShapeDtypeStruct((L, D), f32),
        in_specs=[hbm, vec, vec, hbm, hbm, hbm, hbm, vec, vec, vec, hbm, hbm, hbm],
        out_specs=hbm,
        scratch_shapes=[
            pltpu.VMEM((L, D), bf16),
            pltpu.VMEM((L + 2 * D, D), bf16),
            pltpu.VMEM((2 * P, D), bf16),
            pltpu.VMEM((2, D, P), bf16),
            pltpu.VMEM((L, 2 * P), f32),
            pltpu.VMEM((R, 2 * P), bf16),
            pltpu.VMEM((R, 2 * P), bf16),
            pltpu.VMEM((L, D), f32),
            pltpu.VMEM((G, PB * J, 128), f32),
            pltpu.VMEM((D, F), bf16),
            pltpu.VMEM((D, F), bf16),
            pltpu.VMEM((F, D), bf16),
            pltpu.SemaphoreType.DMA((NB,)),
            pltpu.SemaphoreType.DMA((NA,)),
            pltpu.SemaphoreType.DMA((7,)),
            pltpu.SemaphoreType.DMA((1,)),
        ],
        compiler_params=pltpu.CompilerParams(vmem_limit_bytes=100 * 1024 * 1024),
    )(
        A_x.reshape(L, D),
        A_Lambda_re.reshape(1, P), A_Lambda_im.reshape(1, P),
        A_B_re, A_B_im, A_C_re, A_C_im,
        A_log_dt.reshape(1, P), A_Dskip.reshape(1, D), B_w_r.reshape(1, D),
        B_w_gate, B_w_up, B_w_down,
    )
    return out.reshape(1, L, D)
```

```python
import jax
import jax.numpy as jnp
import numpy as np
import jax.experimental.pallas as pl
import jax.experimental.pallas.tpu as pltpu

L = 2048
D = 1024
P = 1024
F = 3584
NSEG = 8
SEG = L // NSEG
J = 32
NB = SEG // J
R = NSEG * J
G = D // 128
NA = 8
AHEAD = 3
PA = J + 4
PB = 12
NC = 2

_NT = (((1,), (1,)), ((), ()))
f32 = jnp.float32
bf16 = jnp.bfloat16


def _rb(v):
    return v.astype(bf16).astype(f32)


_cur=[None]
def _sc(n):
    if _cur[0] is not None: _cur[0].__exit__(None,None,None)
    _cur[0]=None
    if n:
        _cur[0]=jax.named_scope(n); _cur[0].__enter__()

def _kernel(x_hbm, lre_ref, lim_ref, bre_hbm, bim_hbm, cre_hbm, cim_hbm, ldt_ref,
            dsk_ref, wr_ref, wg_hbm, wu_hbm, wd_hbm, out_hbm,
            x_v, xn_v, b_v, craw_v, bu_v, o_v, st_v, wg_v, wu_v, wd_v,
            sx, sb, sw, so):
    def x_cp(b, s):
        rows = pl.ds(pl.multiple_of(s * SEG + b * J, J), J)
        return pltpu.make_async_copy(x_hbm.at[rows], x_v.at[rows], sx.at[b])

    def b_cp(n):
        return [pltpu.make_async_copy(src.at[pl.ds(n * 128, 128)],
                                      b_v.at[pl.ds(n * 256 + i * 128, 128)], sb.at[n])
                for i, src in enumerate((bre_hbm, bim_hbm))]

    def o_cp(b, s):
        rows = pl.ds(pl.multiple_of(s * SEG + b * J, J), J)
        return pltpu.make_async_copy(o_v.at[rows], out_hbm.at[rows], so.at[0])

    c_cps = [pltpu.make_async_copy(cre_hbm, craw_v.at[0], sw.at[2]),
             pltpu.make_async_copy(cim_hbm, craw_v.at[1], sw.at[3])]
    f_cps = [pltpu.make_async_copy(wg_hbm, wg_v, sw.at[4]),
             pltpu.make_async_copy(wu_hbm, wu_v, sw.at[5]),
             pltpu.make_async_copy(wd_hbm, wd_v, sw.at[6])]

    for b in range(AHEAD):
        for s in range(NSEG):
            x_cp(b, s).start()

    dt = _rb(jnp.exp(ldt_ref[...].astype(f32)))
    lre = lre_ref[...].astype(f32)
    lim = lim_ref[...].astype(f32)
    mag = jnp.exp(dt * lre)
    a_re = mag * jnp.cos(dt * lim)
    a_im = mag * jnp.sin(dt * lim)
    den = lre * lre + lim * lim
    k_re = 2.0 * ((a_re - 1.0) * lre + a_im * lim) / den
    k_im = 2.0 * (a_im * lre - (a_re - 1.0) * lim) / den
    ar8 = jnp.broadcast_to(a_re, (NSEG, P))
    ai8 = jnp.broadcast_to(a_im, (NSEG, P))
    wr = wr_ref[...].astype(f32)
    eps = f32(np.float32(np.asarray(1e-5, dtype=bf16)))

    dsk1 = dsk_ref[...].astype(f32) + 1.0
    lane = jax.lax.broadcasted_iota(jnp.int32, (NSEG, SEG), 1)
    sub = jax.lax.broadcasted_iota(jnp.int32, (NSEG, SEG), 0)

    def norm_rows(b, q, racc):
        x = jnp.concatenate([
            jnp.concatenate([st_v[g, pl.ds(2 * q + j, NSEG, stride=PA), :] for g in range(G)], axis=1)
            for j in range(2)], axis=0)
        m = jnp.sum(x, axis=-1, keepdims=True) * (1.0 / D)
        c = x - m
        v = jnp.sum(c * c, axis=-1, keepdims=True) * (1.0 / D)
        sd = _rb(jnp.sqrt(_rb(_rb(v) + eps)))
        xn = (_rb(x - _rb(m)) * (1.0 / sd)).astype(bf16)
        xn_v[pl.ds(pl.multiple_of(b * R + 16 * q, 16), 16), :] = xn
        r = _rb(jnp.sum(xn.astype(f32) * wr, axis=-1, keepdims=True))
        for j in range(2):
            racc = jnp.where(lane == b * J + 2 * q + j, r[NSEG * j:NSEG * (j + 1), :], racc)
        return racc

    def norm(b, racc):
        for s in range(NSEG):
            x_cp(b, s).wait()

        @pl.when(b + AHEAD < NB)
        def _():
            for s in range(NSEG):
                x_cp(b + AHEAD, s).start()

        for n in range(AHEAD):
            @pl.when(b + AHEAD == NB + n)
            def _():
                for cp in b_cp(n):
                    cp.start()

        for s in range(NSEG):
            nat = pl.ds(pl.multiple_of(s * SEG + b * J, J), J)
            for g in range(G):
                st_v[g, s * PA:s * PA + J, :] = x_v[nat, 128 * g:128 * (g + 1)].astype(f32)
        for q in range(R // 16):
            racc = norm_rows(b, q, racc)
        return racc

    def step(n, h, bu):
        ar, ai = ar8[:, 128 * n:128 * (n + 1)], ai8[:, 128 * n:128 * (n + 1)]
        return (ar * h[0] - ai * h[1] + bu[:, :128], ar * h[1] + ai * h[0] + bu[:, 128:])

    def in_proj(b, n, h):
        rows = pl.ds(pl.multiple_of(b * R, R), R)
        cols = slice(n * 256, (n + 1) * 256)
        bu = jax.lax.dot_general(xn_v[rows, :], b_v[cols, :], _NT, preferred_element_type=f32)
        bu_v[rows, cols] = bu
        for j in range(J):
            h = step(n, h, bu[NSEG * j:NSEG * (j + 1), :])
        return h

    def cprep(row):
        rows = pl.ds(pl.multiple_of(row, 16), 16)
        cre = craw_v[0, rows, :].astype(f32)
        cim = craw_v[1, rows, :].astype(f32)
        xn_v[pl.ds(pl.multiple_of(L + row, 16), 16), :] = (cre * k_re - cim * k_im).astype(bf16)
        xn_v[pl.ds(pl.multiple_of(L + D + row, 16), 16), :] = (cre * (-k_im) - cim * k_re).astype(bf16)

    z = jnp.zeros((NSEG, 128), f32)
    hs = []
    _sc('a0')
    racc = jax.lax.fori_loop(0, NB, norm, jnp.zeros((NSEG, SEG), f32))
    _sc('a1')
    for n in range(NA):
        for cp in b_cp(n):
            cp.wait()
        if n + AHEAD < NA:
            for cp in b_cp(n + AHEAD):
                cp.start()
        if n + AHEAD == NA:
            for cp in c_cps + f_cps:
                cp.start()
        hs.append(in_proj(0, n, (z, z)))
    _sc('aloop')

    def phase_a(b, carry, with_c=False):
        hs = []
        for n in range(NA):
            hs.append(in_proj(b, n, carry[n]))
            if with_c:
                k = 2 * D // NB // NA
                for i in range(k // 16):
                    cprep(((b - NB // 2) * NA + n) * k + 16 * i)
        return hs

    hs = jax.lax.fori_loop(1, NB // 2, phase_a, hs)
    for cp in c_cps:
        cp.wait()
    hs = jax.lax.fori_loop(
        NB // 2, NB, lambda b, c: phase_a(b, c, True), hs)
    _sc('aend')
    er = jnp.concatenate([h[0] for h in hs], axis=1)
    ei = jnp.concatenate([h[1] for h in hs], axis=1)
    _sc('carry')
    pr, pi = ar8, ai8
    n = 1
    while n < SEG:
        pr, pi = pr * pr - pi * pi, 2.0 * pr * pi
        n *= 2
    srow = jax.lax.broadcasted_iota(jnp.int32, (NSEG, P), 0)
    hr = jnp.where(srow >= 1, pltpu.roll(er, 1, 0), 0.0)
    hi = jnp.where(srow >= 1, pltpu.roll(ei, 1, 0), 0.0)
    for sh in (1, 2, 4):
        tr = jnp.where(srow >= sh, pltpu.roll(hr, sh, 0), 0.0)
        ti = jnp.where(srow >= sh, pltpu.roll(hi, sh, 0), 0.0)
        hr, hi = hr + pr * tr - pi * ti, hi + pr * ti + pi * tr
        pr, pi = pr * pr - pi * pi, 2.0 * pr * pi

    _sc('top')
    tok = sub * SEG + lane
    r0 = jnp.max(racc)
    i0 = jnp.min(jnp.where(racc == r0, tok, L))
    rest = jnp.where(tok == i0, -jnp.inf, racc)
    r1 = jnp.max(rest)
    i1 = jnp.min(jnp.where((rest == r1) & (tok != i0), tok, L))
    i0 = jnp.clip(i0, 0, L - 1)
    i1 = jnp.clip(i1, 0, L - 1)
    p0 = (i0 % SEG) * NSEG + i0 // SEG
    p1 = (i1 % SEG) * NSEG + i1 // SEG
    r16 = jax.lax.broadcasted_iota(jnp.int32, (16, D), 0)

    def pick(p):
        g = xn_v[pl.ds(pl.multiple_of((p // 16) * 16, 16), 16), :].astype(f32)
        return jnp.sum(jnp.where(r16 == p % 16, g, 0.0), axis=0, keepdims=True)

    xs = jnp.where(r16 == 0, pick(p0), jnp.where(r16 == 1, pick(p1), 0.0)).astype(bf16)
    _sc('ffn')
    for cp in f_cps:
        cp.wait()
    g = _rb(jnp.dot(xs, wg_v[...], preferred_element_type=f32))
    u = _rb(jnp.dot(xs, wu_v[...], preferred_element_type=f32))
    g = _rb(g * jax.nn.sigmoid(g))
    y = _rb(jnp.dot((g * u).astype(bf16), wd_v[...], preferred_element_type=f32))
    rs = jnp.where(r16 == 0, r0, r1)
    y = _rb(y * _rb(jax.nn.sigmoid(rs)))
    y0 = y[0:1, :]
    y1 = y[1:2, :]
    rowt = jax.lax.broadcasted_iota(jnp.int32, (16, 128), 0)

    def phase_b(b, carry):
        base = pl.multiple_of(b * R, R)
        ys = None
        hs = []
        for n in range(G):
            h = carry[n]
            seq = []
            for j in range(J):
                h = step(n, h, bu_v[pl.ds(base + NSEG * j, NSEG), 256 * n:256 * (n + 1)])
                seq.append(jnp.concatenate(h, axis=1))
            hs.append(h)
            cn = slice(128 * n, 128 * (n + 1))
            cw = jnp.concatenate([xn_v[L:L + D, cn], xn_v[L + D:, cn]], axis=1)
            y = jax.lax.dot_general(jnp.concatenate(seq, axis=0).astype(bf16), cw, _NT,
                                    preferred_element_type=f32)
            ys = y if ys is None else ys + y
        for g in range(G):
            cg = slice(128 * g, 128 * (g + 1))
            for q in range(R // 16):
                row = pl.multiple_of(b * R + 16 * q, 16)
                t = ys[16 * q:16 * (q + 1), cg]
                t = t + xn_v[pl.ds(row, 16), cg].astype(f32) * dsk1[:, cg]
                t = jnp.where(rowt == p0 - row, t + y0[:, cg], t)
                t = jnp.where(rowt == p1 - row, t + y1[:, cg], t)
                for j in range(2):
                    st_v[g, pl.ds(PB * (2 * q + j), 8), :] = t[8 * j:8 * (j + 1), :]
            for s in range(NSEG):
                nat = pl.ds(pl.multiple_of(s * SEG + b * J, J), J)
                o_v[nat, cg] = x_v[nat, cg].astype(f32) + st_v[g, pl.ds(s, J, stride=PB), :]
        for s in range(NSEG):
            o_cp(b, s).start()
        return hs

    _sc('bloop')
    jax.lax.fori_loop(0, NB, phase_b,
                      [(hr[:, 128 * n:128 * (n + 1)], hi[:, 128 * n:128 * (n + 1)]) for n in range(G)])
    _sc('tail')
    pltpu.make_async_copy(o_v, o_v, so.at[0]).wait()
    _sc(None)


@jax.jit
def pallas_parallel_sum__ssm_conv_s5__moe_arch_mod__prompt_kernel(
    A_x: jax.Array,
    A_Lambda_re: jax.Array,
    A_Lambda_im: jax.Array,
    A_B_re: jax.Array,
    A_B_im: jax.Array,
    A_C_re: jax.Array,
    A_C_im: jax.Array,
    A_log_dt: jax.Array,
    A_Dskip: jax.Array,
    B_x: jax.Array,
    B_w_r: jax.Array,
    B_w_gate: jax.Array,
    B_w_up: jax.Array,
    B_w_down: jax.Array,
):
    del B_x
    hbm = pl.BlockSpec(memory_space=pl.ANY)
    vec = pl.BlockSpec(memory_space=pltpu.VMEM)
    out = pl.pallas_call(
        _kernel,
        out_shape=jax.ShapeDtypeStruct((L, D), f32),
        in_specs=[hbm, vec, vec, hbm, hbm, hbm, hbm, vec, vec, vec, hbm, hbm, hbm],
        out_specs=hbm,
        scratch_shapes=[
            pltpu.VMEM((L, D), bf16),
            pltpu.VMEM((L + 2 * D, D), bf16),
            pltpu.VMEM((2 * P, D), bf16),
            pltpu.VMEM((2, D, P), bf16),
            pltpu.VMEM((L, 2 * P), f32),
            pltpu.VMEM((L, D), f32),
            pltpu.VMEM((G, PB * J, 128), f32),
            pltpu.VMEM((D, F), bf16),
            pltpu.VMEM((D, F), bf16),
            pltpu.VMEM((F, D), bf16),
            pltpu.SemaphoreType.DMA((NB,)),
            pltpu.SemaphoreType.DMA((NA,)),
            pltpu.SemaphoreType.DMA((7,)),
            pltpu.SemaphoreType.DMA((1,)),
        ],
        compiler_params=pltpu.CompilerParams(vmem_limit_bytes=100 * 1024 * 1024),
    )(
        A_x.reshape(L, D),
        A_Lambda_re.reshape(1, P), A_Lambda_im.reshape(1, P),
        A_B_re, A_B_im, A_C_re, A_C_im,
        A_log_dt.reshape(1, P), A_Dskip.reshape(1, D), B_w_r.reshape(1, D),
        B_w_gate, B_w_up, B_w_down,
    )
    return out.reshape(1, L, D)
```

```python
import jax
import jax.numpy as jnp
import numpy as np
import jax.experimental.pallas as pl
import jax.experimental.pallas.tpu as pltpu

L = 2048
D = 1024
P = 1024
F = 3584
NSEG = 8
SEG = L // NSEG
J = 32
NB = SEG // J
R = NSEG * J
G = D // 128
NA = 8
AHEAD = 3
PA = J + 4
PB = 12

_NT = (((1,), (1,)), ((), ()))
f32 = jnp.float32
bf16 = jnp.bfloat16


def _rb(v):
    return v.astype(bf16).astype(f32)


def _kernel(x_hbm, lre_ref, lim_ref, bre_hbm, bim_hbm, cre_hbm, cim_hbm, ldt_ref,
            dsk_ref, wr_ref, wg_hbm, wu_hbm, wd_hbm, out_hbm,
            x_v, xn_v, b_v, craw_v, bu_v, o_v, st_v, wg_v, wu_v, wd_v,
            sx, sb, sw, so):
    def x_cp(b, s):
        rows = pl.ds(pl.multiple_of(s * SEG + b * J, J), J)
        return pltpu.make_async_copy(x_hbm.at[rows], x_v.at[rows], sx.at[b])

    def b_cp(n):
        return [pltpu.make_async_copy(src.at[pl.ds(n * 128, 128)],
                                      b_v.at[pl.ds(n * 256 + i * 128, 128)], sb.at[n])
                for i, src in enumerate((bre_hbm, bim_hbm))]

    def o_cp(b, s):
        rows = pl.ds(pl.multiple_of(s * SEG + b * J, J), J)
        return pltpu.make_async_copy(o_v.at[rows], out_hbm.at[rows], so.at[0])

    c_cps = [pltpu.make_async_copy(cre_hbm, craw_v.at[0], sw.at[2]),
             pltpu.make_async_copy(cim_hbm, craw_v.at[1], sw.at[3])]
    f_cps = [pltpu.make_async_copy(wg_hbm, wg_v, sw.at[4]),
             pltpu.make_async_copy(wu_hbm, wu_v, sw.at[5]),
             pltpu.make_async_copy(wd_hbm, wd_v, sw.at[6])]

    for b in range(AHEAD):
        for s in range(NSEG):
            x_cp(b, s).start()

    dt = _rb(jnp.exp(ldt_ref[...].astype(f32)))
    lre = lre_ref[...].astype(f32)
    lim = lim_ref[...].astype(f32)
    mag = jnp.exp(dt * lre)
    a_re = mag * jnp.cos(dt * lim)
    a_im = mag * jnp.sin(dt * lim)
    den = lre * lre + lim * lim
    k_re = 2.0 * ((a_re - 1.0) * lre + a_im * lim) / den
    k_im = 2.0 * (a_im * lre - (a_re - 1.0) * lim) / den
    ar8 = jnp.broadcast_to(a_re, (NSEG, P))
    ai8 = jnp.broadcast_to(a_im, (NSEG, P))
    wr = wr_ref[...].astype(f32)
    eps = f32(np.float32(np.asarray(1e-5, dtype=bf16)))

    dsk1 = dsk_ref[...].astype(f32) + 1.0
    lane = jax.lax.broadcasted_iota(jnp.int32, (NSEG, SEG), 1)
    sub = jax.lax.broadcasted_iota(jnp.int32, (NSEG, SEG), 0)

    def norm_rows(b, q, racc):
        x = jnp.concatenate([
            jnp.concatenate([st_v[g, pl.ds(2 * q + j, NSEG, stride=PA), :] for g in range(G)], axis=1)
            for j in range(2)], axis=0)
        m = jnp.sum(x, axis=-1, keepdims=True) * (1.0 / D)
        c = x - m
        v = jnp.sum(c * c, axis=-1, keepdims=True) * (1.0 / D)
        sd = _rb(jnp.sqrt(_rb(_rb(v) + eps)))
        xn = (_rb(x - _rb(m)) * (1.0 / sd)).astype(bf16)
        xn_v[pl.ds(pl.multiple_of(b * R + 16 * q, 16), 16), :] = xn
        r = _rb(jnp.sum(xn.astype(f32) * wr, axis=-1, keepdims=True))
        for j in range(2):
            racc = jnp.where(lane == b * J + 2 * q + j, r[NSEG * j:NSEG * (j + 1), :], racc)
        return racc

    def norm(b, racc):
        for s in range(NSEG):
            x_cp(b, s).wait()

        @pl.when(b + AHEAD < NB)
        def _():
            for s in range(NSEG):
                x_cp(b + AHEAD, s).start()

        for n in range(AHEAD):
            @pl.when(b + AHEAD == NB + n)
            def _():
                for cp in b_cp(n):
                    cp.start()

        for s in range(NSEG):
            nat = pl.ds(pl.multiple_of(s * SEG + b * J, J), J)
            for g in range(G):
                st_v[g, s * PA:s * PA + J, :] = x_v[nat, 128 * g:128 * (g + 1)].astype(f32)
        for q in range(R // 16):
            racc = norm_rows(b, q, racc)
        return racc

    def step(n, h, bu):
        ar, ai = ar8[:, 128 * n:128 * (n + 1)], ai8[:, 128 * n:128 * (n + 1)]
        return (ar * h[0] - ai * h[1] + bu[:, :128], ar * h[1] + ai * h[0] + bu[:, 128:])

    def in_proj(b, n, h):
        rows = pl.ds(pl.multiple_of(b * R, R), R)
        cols = slice(n * 256, (n + 1) * 256)
        bu = jax.lax.dot_general(xn_v[rows, :], b_v[cols, :], _NT, preferred_element_type=f32)
        bu_v[rows, cols] = bu
        for j in range(J):
            h = step(n, h, bu[NSEG * j:NSEG * (j + 1), :])
        return h

    def cprep(row):
        rows = pl.ds(pl.multiple_of(row, 16), 16)
        cre = craw_v[0, rows, :].astype(f32)
        cim = craw_v[1, rows, :].astype(f32)
        xn_v[pl.ds(pl.multiple_of(L + row, 16), 16), :] = (cre * k_re - cim * k_im).astype(bf16)
        xn_v[pl.ds(pl.multiple_of(L + D + row, 16), 16), :] = (cre * (-k_im) - cim * k_re).astype(bf16)

    z = jnp.zeros((NSEG, 128), f32)
    hs = []
    racc = jax.lax.fori_loop(0, NB, norm, jnp.zeros((NSEG, SEG), f32))
    for n in range(NA):
        for cp in b_cp(n):
            cp.wait()
        if n + AHEAD < NA:
            for cp in b_cp(n + AHEAD):
                cp.start()
        if n + AHEAD == NA:
            for cp in c_cps + f_cps:
                cp.start()
        hs.append(in_proj(0, n, (z, z)))

    def phase_a(b, carry, with_c=False):
        hs = []
        for n in range(NA):
            hs.append(in_proj(b, n, carry[n]))
            if with_c:
                k = 2 * D // NB // NA
                for i in range(k // 16):
                    cprep(((b - NB // 2) * NA + n) * k + 16 * i)
        return hs

    hs = jax.lax.fori_loop(1, NB // 2, phase_a, hs)
    for cp in c_cps:
        cp.wait()
    hs = jax.lax.fori_loop(
        NB // 2, NB, lambda b, c: phase_a(b, c, True), hs)
    er = jnp.concatenate([h[0] for h in hs], axis=1)
    ei = jnp.concatenate([h[1] for h in hs], axis=1)
    pr, pi = ar8, ai8
    n = 1
    while n < SEG:
        pr, pi = pr * pr - pi * pi, 2.0 * pr * pi
        n *= 2
    srow = jax.lax.broadcasted_iota(jnp.int32, (NSEG, P), 0)
    hr = jnp.where(srow >= 1, pltpu.roll(er, 1, 0), 0.0)
    hi = jnp.where(srow >= 1, pltpu.roll(ei, 1, 0), 0.0)
    for sh in (1, 2, 4):
        tr = jnp.where(srow >= sh, pltpu.roll(hr, sh, 0), 0.0)
        ti = jnp.where(srow >= sh, pltpu.roll(hi, sh, 0), 0.0)
        hr, hi = hr + pr * tr - pi * ti, hi + pr * ti + pi * tr
        pr, pi = pr * pr - pi * pi, 2.0 * pr * pi

    tok = sub * SEG + lane
    r0 = jnp.max(racc)
    i0 = jnp.min(jnp.where(racc == r0, tok, L))
    rest = jnp.where(tok == i0, -jnp.inf, racc)
    r1 = jnp.max(rest)
    i1 = jnp.min(jnp.where((rest == r1) & (tok != i0), tok, L))
    i0 = jnp.clip(i0, 0, L - 1)
    i1 = jnp.clip(i1, 0, L - 1)
    p0 = (i0 % SEG) * NSEG + i0 // SEG
    p1 = (i1 % SEG) * NSEG + i1 // SEG
    r16 = jax.lax.broadcasted_iota(jnp.int32, (16, D), 0)

    def pick(p):
        g = xn_v[pl.ds(pl.multiple_of((p // 16) * 16, 16), 16), :].astype(f32)
        return jnp.sum(jnp.where(r16 == p % 16, g, 0.0), axis=0, keepdims=True)

    xs = jnp.where(r16 == 0, pick(p0), jnp.where(r16 == 1, pick(p1), 0.0)).astype(bf16)
    for cp in f_cps:
        cp.wait()
    g = _rb(jnp.dot(xs, wg_v[...], preferred_element_type=f32))
    u = _rb(jnp.dot(xs, wu_v[...], preferred_element_type=f32))
    g = _rb(g * jax.nn.sigmoid(g))
    y = _rb(jnp.dot((g * u).astype(bf16), wd_v[...], preferred_element_type=f32))
    rs = jnp.where(r16 == 0, r0, r1)
    y = _rb(y * _rb(jax.nn.sigmoid(rs)))
    y0 = y[0:1, :]
    y1 = y[1:2, :]
    rowt = jax.lax.broadcasted_iota(jnp.int32, (16, 128), 0)

    def phase_b(b, carry):
        base = pl.multiple_of(b * R, R)
        ys = None
        hs = []
        for n in range(G):
            h = carry[n]
            seq = []
            for j in range(J):
                h = step(n, h, bu_v[pl.ds(base + NSEG * j, NSEG), 256 * n:256 * (n + 1)])
                seq.append(jnp.concatenate(h, axis=1))
            hs.append(h)
            cn = slice(128 * n, 128 * (n + 1))
            cw = jnp.concatenate([xn_v[L:L + D, cn], xn_v[L + D:, cn]], axis=1)
            y = jax.lax.dot_general(jnp.concatenate(seq, axis=0).astype(bf16), cw, _NT,
                                    preferred_element_type=f32)
            ys = y if ys is None else ys + y
        for g in range(G):
            cg = slice(128 * g, 128 * (g + 1))
            for q in range(R // 16):
                row = pl.multiple_of(b * R + 16 * q, 16)
                t = ys[16 * q:16 * (q + 1), cg]
                t = t + xn_v[pl.ds(row, 16), cg].astype(f32) * dsk1[:, cg]
                t = jnp.where(rowt == p0 - row, t + y0[:, cg], t)
                t = jnp.where(rowt == p1 - row, t + y1[:, cg], t)
                for j in range(2):
                    st_v[g, pl.ds(PB * (2 * q + j), 8), :] = t[8 * j:8 * (j + 1), :]
            for s in range(NSEG):
                nat = pl.ds(pl.multiple_of(s * SEG + b * J, J), J)
                o_v[nat, cg] = x_v[nat, cg].astype(f32) + st_v[g, pl.ds(s, J, stride=PB), :]
        for s in range(NSEG):
            o_cp(b, s).start()
        return hs

    jax.lax.fori_loop(0, NB, phase_b,
                      [(hr[:, 128 * n:128 * (n + 1)], hi[:, 128 * n:128 * (n + 1)]) for n in range(G)])
    pltpu.make_async_copy(o_v, o_v, so.at[0]).wait()


@jax.jit
def pallas_parallel_sum__ssm_conv_s5__moe_arch_mod__prompt_kernel(
    A_x: jax.Array,
    A_Lambda_re: jax.Array,
    A_Lambda_im: jax.Array,
    A_B_re: jax.Array,
    A_B_im: jax.Array,
    A_C_re: jax.Array,
    A_C_im: jax.Array,
    A_log_dt: jax.Array,
    A_Dskip: jax.Array,
    B_x: jax.Array,
    B_w_r: jax.Array,
    B_w_gate: jax.Array,
    B_w_up: jax.Array,
    B_w_down: jax.Array,
):
    del B_x
    hbm = pl.BlockSpec(memory_space=pl.ANY)
    vec = pl.BlockSpec(memory_space=pltpu.VMEM)
    out = pl.pallas_call(
        _kernel,
        out_shape=jax.ShapeDtypeStruct((L, D), f32),
        in_specs=[hbm, vec, vec, hbm, hbm, hbm, hbm, vec, vec, vec, hbm, hbm, hbm],
        out_specs=hbm,
        scratch_shapes=[
            pltpu.VMEM((L, D), bf16),
            pltpu.VMEM((L + 2 * D, D), bf16),
            pltpu.VMEM((2 * P, D), bf16),
            pltpu.VMEM((2, D, P), bf16),
            pltpu.VMEM((L, 2 * P), f32),
            pltpu.VMEM((L, D), f32),
            pltpu.VMEM((G, PB * J, 128), f32),
            pltpu.VMEM((D, F), bf16),
            pltpu.VMEM((D, F), bf16),
            pltpu.VMEM((F, D), bf16),
            pltpu.SemaphoreType.DMA((NB,)),
            pltpu.SemaphoreType.DMA((NA,)),
            pltpu.SemaphoreType.DMA((7,)),
            pltpu.SemaphoreType.DMA((1,)),
        ],
        compiler_params=pltpu.CompilerParams(vmem_limit_bytes=100 * 1024 * 1024),
    )(
        A_x.reshape(L, D),
        A_Lambda_re.reshape(1, P), A_Lambda_im.reshape(1, P),
        A_B_re, A_B_im, A_C_re, A_C_im,
        A_log_dt.reshape(1, P), A_Dskip.reshape(1, D), B_w_r.reshape(1, D),
        B_w_gate, B_w_up, B_w_down,
    )
    return out.reshape(1, L, D)
```

```python
import jax
import jax.numpy as jnp
import numpy as np
import jax.experimental.pallas as pl
import jax.experimental.pallas.tpu as pltpu

L = 2048
D = 1024
P = 1024
F = 3584
NSEG = 8
SEG = L // NSEG
J = 32
NB = SEG // J
R = NSEG * J
G = D // 128
NA = 8
AHEAD = 3
PA = J + 4
PB = 12

_NT = (((1,), (1,)), ((), ()))
f32 = jnp.float32
bf16 = jnp.bfloat16


def _rb(v):
    return v.astype(bf16).astype(f32)


def _kernel(x_hbm, lre_ref, lim_ref, bre_hbm, bim_hbm, cre_hbm, cim_hbm, ldt_ref,
            dsk_ref, wr_ref, wg_hbm, wu_hbm, wd_hbm, out_hbm,
            x_v, xn_v, b_v, craw_v, bu_v, o_v, st_v, wg_v, wu_v, wd_v,
            sx, sb, sw, so):
    def x_cp(b, s):
        rows = pl.ds(pl.multiple_of(s * SEG + b * J, J), J)
        return pltpu.make_async_copy(x_hbm.at[rows], x_v.at[rows], sx.at[b])

    def b_cp(n):
        return [pltpu.make_async_copy(src.at[pl.ds(n * 128, 128)],
                                      b_v.at[pl.ds(n * 256 + i * 128, 128)], sb.at[n])
                for i, src in enumerate((bre_hbm, bim_hbm))]

    def o_cp(b, s):
        rows = pl.ds(pl.multiple_of(s * SEG + b * J, J), J)
        return pltpu.make_async_copy(o_v.at[rows], out_hbm.at[rows], so.at[0])

    c_cps = [pltpu.make_async_copy(cre_hbm, craw_v.at[0], sw.at[2]),
             pltpu.make_async_copy(cim_hbm, craw_v.at[1], sw.at[3])]
    f_cps = [pltpu.make_async_copy(wg_hbm, wg_v, sw.at[4]),
             pltpu.make_async_copy(wu_hbm, wu_v, sw.at[5]),
             pltpu.make_async_copy(wd_hbm, wd_v, sw.at[6])]

    for b in range(AHEAD):
        for s in range(NSEG):
            x_cp(b, s).start()

    dt = _rb(jnp.exp(ldt_ref[...].astype(f32).reshape(1, D)))
    lre = lre_ref[...].astype(f32).reshape(1, D)
    lim = lim_ref[...].astype(f32).reshape(1, D)
    mag = jnp.exp(dt * lre)
    a_re = mag * jnp.cos(dt * lim)
    a_im = mag * jnp.sin(dt * lim)
    den = lre * lre + lim * lim
    k_re = 2.0 * ((a_re - 1.0) * lre + a_im * lim) / den
    k_im = 2.0 * (a_im * lre - (a_re - 1.0) * lim) / den
    ar8 = jnp.broadcast_to(a_re, (NSEG, P))
    ai8 = jnp.broadcast_to(a_im, (NSEG, P))
    wr = wr_ref[...].astype(f32).reshape(1, D)
    eps = f32(np.float32(np.asarray(1e-5, dtype=bf16)))

    dsk1 = dsk_ref[...].astype(f32).reshape(1, D) + 1.0
    lane = jax.lax.broadcasted_iota(jnp.int32, (NSEG, SEG), 1)
    sub = jax.lax.broadcasted_iota(jnp.int32, (NSEG, SEG), 0)

    def norm_rows(b, q, racc):
        x = jnp.concatenate([
            jnp.concatenate([st_v[g, pl.ds(2 * q + j, NSEG, stride=PA), :] for g in range(G)], axis=1)
            for j in range(2)], axis=0)
        m = jnp.sum(x, axis=-1, keepdims=True) * (1.0 / D)
        c = x - m
        v = jnp.sum(c * c, axis=-1, keepdims=True) * (1.0 / D)
        sd = _rb(jnp.sqrt(_rb(_rb(v) + eps)))
        xn = (_rb(x - _rb(m)) * (1.0 / sd)).astype(bf16)
        xn_v[pl.ds(pl.multiple_of(b * R + 16 * q, 16), 16), :] = xn
        r = _rb(jnp.sum(xn.astype(f32) * wr, axis=-1, keepdims=True))
        for j in range(2):
            racc = jnp.where(lane == b * J + 2 * q + j, r[NSEG * j:NSEG * (j + 1), :], racc)
        return racc

    def norm(b, racc):
        for s in range(NSEG):
            x_cp(b, s).wait()

        @pl.when(b + AHEAD < NB)
        def _():
            for s in range(NSEG):
                x_cp(b + AHEAD, s).start()

        for n in range(AHEAD):
            @pl.when(b + AHEAD == NB + n)
            def _():
                for cp in b_cp(n):
                    cp.start()

        for s in range(NSEG):
            nat = pl.ds(pl.multiple_of(s * SEG + b * J, J), J)
            for g in range(G):
                st_v[g, s * PA:s * PA + J, :] = x_v[nat, 128 * g:128 * (g + 1)].astype(f32)
        for q in range(R // 16):
            racc = norm_rows(b, q, racc)
        return racc

    def step(n, h, bu):
        ar, ai = ar8[:, 128 * n:128 * (n + 1)], ai8[:, 128 * n:128 * (n + 1)]
        return (ar * h[0] - ai * h[1] + bu[:, :128], ar * h[1] + ai * h[0] + bu[:, 128:])

    def in_proj(b, n, h):
        rows = pl.ds(pl.multiple_of(b * R, R), R)
        cols = slice(n * 256, (n + 1) * 256)
        bu = jax.lax.dot_general(xn_v[rows, :], b_v[cols, :], _NT, preferred_element_type=f32)
        bu_v[rows, cols] = bu
        for j in range(J):
            h = step(n, h, bu[NSEG * j:NSEG * (j + 1), :])
        return h

    def cprep(row):
        rows = pl.ds(pl.multiple_of(row, 16), 16)
        cre = craw_v[0, rows, :].astype(f32)
        cim = craw_v[1, rows, :].astype(f32)
        xn_v[pl.ds(pl.multiple_of(L + row, 16), 16), :] = (cre * k_re - cim * k_im).astype(bf16)
        xn_v[pl.ds(pl.multiple_of(L + D + row, 16), 16), :] = (cre * (-k_im) - cim * k_re).astype(bf16)

    z = jnp.zeros((NSEG, 128), f32)
    hs = []
    racc = jax.lax.fori_loop(0, NB, norm, jnp.zeros((NSEG, SEG), f32))
    for n in range(NA):
        for cp in b_cp(n):
            cp.wait()
        if n + AHEAD < NA:
            for cp in b_cp(n + AHEAD):
                cp.start()
        if n + AHEAD == NA:
            for cp in c_cps + f_cps:
                cp.start()
        hs.append(in_proj(0, n, (z, z)))

    def phase_a(b, carry, with_c=False):
        hs = []
        for n in range(NA):
            hs.append(in_proj(b, n, carry[n]))
            if with_c:
                k = 2 * D // NB // NA
                for i in range(k // 16):
                    cprep(((b - NB // 2) * NA + n) * k + 16 * i)
        return hs

    hs = jax.lax.fori_loop(1, NB // 2, phase_a, hs)
    for cp in c_cps:
        cp.wait()
    hs = jax.lax.fori_loop(
        NB // 2, NB, lambda b, c: phase_a(b, c, True), hs)
    er = jnp.concatenate([h[0] for h in hs], axis=1)
    ei = jnp.concatenate([h[1] for h in hs], axis=1)
    pr, pi = ar8, ai8
    n = 1
    while n < SEG:
        pr, pi = pr * pr - pi * pi, 2.0 * pr * pi
        n *= 2
    srow = jax.lax.broadcasted_iota(jnp.int32, (NSEG, P), 0)
    hr = jnp.where(srow >= 1, pltpu.roll(er, 1, 0), 0.0)
    hi = jnp.where(srow >= 1, pltpu.roll(ei, 1, 0), 0.0)
    for sh in (1, 2, 4):
        tr = jnp.where(srow >= sh, pltpu.roll(hr, sh, 0), 0.0)
        ti = jnp.where(srow >= sh, pltpu.roll(hi, sh, 0), 0.0)
        hr, hi = hr + pr * tr - pi * ti, hi + pr * ti + pi * tr
        pr, pi = pr * pr - pi * pi, 2.0 * pr * pi

    tok = sub * SEG + lane
    r0 = jnp.max(racc)
    i0 = jnp.min(jnp.where(racc == r0, tok, L))
    rest = jnp.where(tok == i0, -jnp.inf, racc)
    r1 = jnp.max(rest)
    i1 = jnp.min(jnp.where((rest == r1) & (tok != i0), tok, L))
    i0 = jnp.clip(i0, 0, L - 1)
    i1 = jnp.clip(i1, 0, L - 1)
    p0 = (i0 % SEG) * NSEG + i0 // SEG
    p1 = (i1 % SEG) * NSEG + i1 // SEG
    r16 = jax.lax.broadcasted_iota(jnp.int32, (16, D), 0)

    def pick(p):
        g = xn_v[pl.ds(pl.multiple_of((p // 16) * 16, 16), 16), :].astype(f32)
        return jnp.sum(jnp.where(r16 == p % 16, g, 0.0), axis=0, keepdims=True)

    xs = jnp.where(r16 == 0, pick(p0), jnp.where(r16 == 1, pick(p1), 0.0)).astype(bf16)
    for cp in f_cps:
        cp.wait()
    g = _rb(jnp.dot(xs, wg_v[...], preferred_element_type=f32))
    u = _rb(jnp.dot(xs, wu_v[...], preferred_element_type=f32))
    g = _rb(g * jax.nn.sigmoid(g))
    y = _rb(jnp.dot((g * u).astype(bf16), wd_v[...], preferred_element_type=f32))
    rs = jnp.where(r16 == 0, r0, r1)
    y = _rb(y * _rb(jax.nn.sigmoid(rs)))
    y0 = y[0:1, :]
    y1 = y[1:2, :]
    rowt = jax.lax.broadcasted_iota(jnp.int32, (16, 128), 0)

    def phase_b(b, carry):
        base = pl.multiple_of(b * R, R)
        ys = None
        hs = []
        for n in range(G):
            h = carry[n]
            seq = []
            for j in range(J):
                h = step(n, h, bu_v[pl.ds(base + NSEG * j, NSEG), 256 * n:256 * (n + 1)])
                seq.append(jnp.concatenate(h, axis=1))
            hs.append(h)
            cn = slice(128 * n, 128 * (n + 1))
            cw = jnp.concatenate([xn_v[L:L + D, cn], xn_v[L + D:, cn]], axis=1)
            y = jax.lax.dot_general(jnp.concatenate(seq, axis=0).astype(bf16), cw, _NT,
                                    preferred_element_type=f32)
            ys = y if ys is None else ys + y
        for g in range(G):
            cg = slice(128 * g, 128 * (g + 1))
            for q in range(R // 16):
                row = pl.multiple_of(b * R + 16 * q, 16)
                t = ys[16 * q:16 * (q + 1), cg]
                t = t + xn_v[pl.ds(row, 16), cg].astype(f32) * dsk1[:, cg]
                t = jnp.where(rowt == p0 - row, t + y0[:, cg], t)
                t = jnp.where(rowt == p1 - row, t + y1[:, cg], t)
                for j in range(2):
                    st_v[g, pl.ds(PB * (2 * q + j), 8), :] = t[8 * j:8 * (j + 1), :]
            for s in range(NSEG):
                nat = pl.ds(pl.multiple_of(s * SEG + b * J, J), J)
                o_v[nat, cg] = x_v[nat, cg].astype(f32) + st_v[g, pl.ds(s, J, stride=PB), :]
        for s in range(NSEG):
            o_cp(b, s).start()
        return hs

    jax.lax.fori_loop(0, NB, phase_b,
                      [(hr[:, 128 * n:128 * (n + 1)], hi[:, 128 * n:128 * (n + 1)]) for n in range(G)])
    pltpu.make_async_copy(o_v, o_v, so.at[0]).wait()


@jax.jit
def pallas_parallel_sum__ssm_conv_s5__moe_arch_mod__prompt_kernel(
    A_x: jax.Array,
    A_Lambda_re: jax.Array,
    A_Lambda_im: jax.Array,
    A_B_re: jax.Array,
    A_B_im: jax.Array,
    A_C_re: jax.Array,
    A_C_im: jax.Array,
    A_log_dt: jax.Array,
    A_Dskip: jax.Array,
    B_x: jax.Array,
    B_w_r: jax.Array,
    B_w_gate: jax.Array,
    B_w_up: jax.Array,
    B_w_down: jax.Array,
):
    del B_x
    hbm = pl.BlockSpec(memory_space=pl.ANY)
    vec = pl.BlockSpec(memory_space=pltpu.VMEM)
    out = pl.pallas_call(
        _kernel,
        out_shape=jax.ShapeDtypeStruct((L, D), f32),
        in_specs=[hbm, vec, vec, hbm, hbm, hbm, hbm, vec, vec, vec, hbm, hbm, hbm],
        out_specs=hbm,
        scratch_shapes=[
            pltpu.VMEM((L, D), bf16),
            pltpu.VMEM((L + 2 * D, D), bf16),
            pltpu.VMEM((2 * P, D), bf16),
            pltpu.VMEM((2, D, P), bf16),
            pltpu.VMEM((L, 2 * P), f32),
            pltpu.VMEM((L, D), f32),
            pltpu.VMEM((G, PB * J, 128), f32),
            pltpu.VMEM((D, F), bf16),
            pltpu.VMEM((D, F), bf16),
            pltpu.VMEM((F, D), bf16),
            pltpu.SemaphoreType.DMA((NB,)),
            pltpu.SemaphoreType.DMA((NA,)),
            pltpu.SemaphoreType.DMA((7,)),
            pltpu.SemaphoreType.DMA((1,)),
        ],
        compiler_params=pltpu.CompilerParams(vmem_limit_bytes=100 * 1024 * 1024),
    )(
        A_x.reshape(L, D),
        A_Lambda_re, A_Lambda_im,
        A_B_re, A_B_im, A_C_re, A_C_im,
        A_log_dt, A_Dskip, B_w_r,
        B_w_gate, B_w_up, B_w_down,
    )
    return out.reshape(1, L, D)
```

```python
import jax
import jax.numpy as jnp
import numpy as np
import jax.experimental.pallas as pl
import jax.experimental.pallas.tpu as pltpu

L = 2048
D = 1024
P = 1024
F = 3584
NSEG = 8
SEG = L // NSEG
J = 32
NB = SEG // J
R = NSEG * J
G = D // 128
NA = 8
AHEAD = 3
PA = J + 4
PB = 12

_NT = (((1,), (1,)), ((), ()))
f32 = jnp.float32
bf16 = jnp.bfloat16


def _rb(v):
    return v.astype(bf16).astype(f32)


def _kernel(x_hbm, lre_ref, lim_ref, bre_hbm, bim_hbm, cre_hbm, cim_hbm, ldt_ref,
            dsk_ref, wr_ref, wg_hbm, wu_hbm, wd_hbm, out_hbm,
            x_v, xn_v, b_v, craw_v, bu_v, o_v, st_v, wg_v, wu_v, wd_v,
            sx, sb, sw, so):
    def x_cp(b, s):
        rows = pl.ds(pl.multiple_of(s * SEG + b * J, J), J)
        return pltpu.make_async_copy(x_hbm.at[rows], x_v.at[rows], sx.at[b])

    def b_cp(n):
        return [pltpu.make_async_copy(src.at[pl.ds(n * 128, 128)],
                                      b_v.at[pl.ds(n * 256 + i * 128, 128)], sb.at[n])
                for i, src in enumerate((bre_hbm, bim_hbm))]

    def o_cp(b, s):
        rows = pl.ds(pl.multiple_of(s * SEG + b * J, J), J)
        return pltpu.make_async_copy(o_v.at[rows], out_hbm.at[rows], so.at[0])

    c_cps = [pltpu.make_async_copy(cre_hbm, craw_v.at[0], sw.at[2]),
             pltpu.make_async_copy(cim_hbm, craw_v.at[1], sw.at[3])]
    f_cps = [pltpu.make_async_copy(wg_hbm, wg_v, sw.at[4]),
             pltpu.make_async_copy(wu_hbm, wu_v, sw.at[5]),
             pltpu.make_async_copy(wd_hbm, wd_v, sw.at[6])]

    for b in range(1):
        for s in range(NSEG):
            x_cp(b, s).start()

    dt = _rb(jnp.exp(ldt_ref[...].astype(f32).reshape(1, D)))
    lre = lre_ref[...].astype(f32).reshape(1, D)
    lim = lim_ref[...].astype(f32).reshape(1, D)
    mag = jnp.exp(dt * lre)
    a_re = mag * jnp.cos(dt * lim)
    a_im = mag * jnp.sin(dt * lim)
    den = lre * lre + lim * lim
    k_re = 2.0 * ((a_re - 1.0) * lre + a_im * lim) / den
    k_im = 2.0 * (a_im * lre - (a_re - 1.0) * lim) / den
    ar8 = jnp.broadcast_to(a_re, (NSEG, P))
    ai8 = jnp.broadcast_to(a_im, (NSEG, P))
    wr = wr_ref[...].astype(f32).reshape(1, D)
    eps = f32(np.float32(np.asarray(1e-5, dtype=bf16)))

    dsk1 = dsk_ref[...].astype(f32).reshape(1, D) + 1.0
    lane = jax.lax.broadcasted_iota(jnp.int32, (NSEG, SEG), 1)
    sub = jax.lax.broadcasted_iota(jnp.int32, (NSEG, SEG), 0)

    def tie(v, z):
        return v if z is None else pltpu.bitcast(pltpu.bitcast(v, jnp.int32) | z, f32)

    def norm_rows(b, q, racc, z=None):
        x = jnp.concatenate([
            jnp.concatenate([tie(st_v[g, pl.ds(2 * q + j, NSEG, stride=PA), :], z if g == 0 else None) for g in range(G)], axis=1)
            for j in range(2)], axis=0)
        m = jnp.sum(x, axis=-1, keepdims=True) * (1.0 / D)
        c = x - m
        v = jnp.sum(c * c, axis=-1, keepdims=True) * (1.0 / D)
        sd = _rb(jnp.sqrt(_rb(_rb(v) + eps)))
        xn = (_rb(x - _rb(m)) * (1.0 / sd)).astype(bf16)
        xn_v[pl.ds(pl.multiple_of(b * R + 16 * q, 16), 16), :] = xn
        r = _rb(jnp.sum(xn.astype(f32) * wr, axis=-1, keepdims=True))
        for j in range(2):
            racc = jnp.where(lane == b * J + 2 * q + j, r[NSEG * j:NSEG * (j + 1), :], racc)
        return racc

    def stage(b, s, z=None):
        nat = pl.ds(pl.multiple_of(s * SEG + b * J, J), J)
        for g in range(G):
            zz = None if z is None else jnp.concatenate([z] * (J // 8), axis=0)
            st_v[g, s * PA:s * PA + J, :] = tie(x_v[nat, 128 * g:128 * (g + 1)].astype(f32), zz)

    def step(n, h, bu):
        ar, ai = ar8[:, 128 * n:128 * (n + 1)], ai8[:, 128 * n:128 * (n + 1)]
        return (ar * h[0] - ai * h[1] + bu[:, :128], ar * h[1] + ai * h[0] + bu[:, 128:])

    def in_proj(b, n, h):
        rows = pl.ds(pl.multiple_of(b * R, R), R)
        cols = slice(n * 256, (n + 1) * 256)
        bu = jax.lax.dot_general(xn_v[rows, :], b_v[cols, :], _NT, preferred_element_type=f32)
        bu_v[rows, cols] = bu
        for j in range(J):
            h = step(n, h, bu[NSEG * j:NSEG * (j + 1), :])
        t = pltpu.bitcast(bu[:, :128], jnp.int32)
        zs = [(t[8 * i:8 * i + 8] * t[8 * i:8 * i + 8]) & 2 for i in range(0, J, J // 4)]
        return h, zs

    def cprep(row):
        rows = pl.ds(pl.multiple_of(row, 16), 16)
        cre = craw_v[0, rows, :].astype(f32)
        cim = craw_v[1, rows, :].astype(f32)
        xn_v[pl.ds(pl.multiple_of(L + row, 16), 16), :] = (cre * k_re - cim * k_im).astype(bf16)
        xn_v[pl.ds(pl.multiple_of(L + D + row, 16), 16), :] = (cre * (-k_im) - cim * k_re).astype(bf16)

    z = jnp.zeros((NSEG, 128), f32)
    hs = []
    for n in range(AHEAD):
        for cp in b_cp(n):
            cp.start()
    for s in range(NSEG):
        x_cp(0, s).wait()
        stage(0, s)
    racc = jnp.zeros((NSEG, SEG), f32)
    for q in range(R // 16):
        racc = norm_rows(0, q, racc)

    def phase_a(b, carry, with_c=False, first=False, last=False):
        hp, racc = carry
        hs = []
        for n in range(NA):
            if first:
                for cp in b_cp(n):
                    cp.wait()
                if n + AHEAD < NA:
                    for cp in b_cp(n + AHEAD):
                        cp.start()
                for s in range(NSEG):
                    if n == 1:
                        x_cp(1, s).start()
                    if n == 4:
                        x_cp(1, s).wait()
                    if n == NA - AHEAD:
                        for bb in range(2, NB):
                            x_cp(bb, s).start()
            h, zs = in_proj(b, n, hp[n])
            hs.append(h)
            if not last and not first:
                if n < 2:
                    for i in range(4):
                        stage(b + 1, 4 * n + i, zs[i])
                else:
                    qs = range((n - 2) * 16 // 6, (n - 1) * 16 // 6)
                    for i, q in enumerate(qs):
                        racc = norm_rows(b + 1, q, racc, zs[i])
            if first and n == 4:
                for i in range(8):
                    stage(1, i, zs[i // 2])
            if first and n > 4:
                for i, q in enumerate(range((n - 5) * 16 // 3, (n - 4) * 16 // 3)):
                    racc = norm_rows(1, q, racc, zs[i % 4])
            if with_c:
                k = 2 * D // NB // NA
                for i in range(k // 16):
                    cprep(((b - NB // 2) * NA + n) * k + 16 * i)
        return hs, racc

    hs, racc = phase_a(0, ([(z, z)] * NA, racc), first=True)
    for bb in range(2, NB):
        for s in range(NSEG):
            x_cp(bb, s).wait()
    for cp in c_cps + f_cps:
        cp.start()
    hs = jax.lax.fori_loop(1, NB // 2, phase_a, (hs, racc))
    for cp in c_cps:
        cp.wait()
    hs = jax.lax.fori_loop(
        NB // 2, NB - 1, lambda b, c: phase_a(b, c, True), hs)
    hs, racc = phase_a(NB - 1, hs, True, last=True)
    er = jnp.concatenate([h[0] for h in hs], axis=1)
    ei = jnp.concatenate([h[1] for h in hs], axis=1)
    pr, pi = ar8, ai8
    n = 1
    while n < SEG:
        pr, pi = pr * pr - pi * pi, 2.0 * pr * pi
        n *= 2
    srow = jax.lax.broadcasted_iota(jnp.int32, (NSEG, P), 0)
    hr = jnp.where(srow >= 1, pltpu.roll(er, 1, 0), 0.0)
    hi = jnp.where(srow >= 1, pltpu.roll(ei, 1, 0), 0.0)
    for sh in (1, 2, 4):
        tr = jnp.where(srow >= sh, pltpu.roll(hr, sh, 0), 0.0)
        ti = jnp.where(srow >= sh, pltpu.roll(hi, sh, 0), 0.0)
        hr, hi = hr + pr * tr - pi * ti, hi + pr * ti + pi * tr
        pr, pi = pr * pr - pi * pi, 2.0 * pr * pi

    tok = sub * SEG + lane
    r0 = jnp.max(racc)
    i0 = jnp.min(jnp.where(racc == r0, tok, L))
    rest = jnp.where(tok == i0, -jnp.inf, racc)
    r1 = jnp.max(rest)
    i1 = jnp.min(jnp.where((rest == r1) & (tok != i0), tok, L))
    i0 = jnp.clip(i0, 0, L - 1)
    i1 = jnp.clip(i1, 0, L - 1)
    p0 = (i0 % SEG) * NSEG + i0 // SEG
    p1 = (i1 % SEG) * NSEG + i1 // SEG
    r16 = jax.lax.broadcasted_iota(jnp.int32, (16, D), 0)

    def pick(p):
        g = xn_v[pl.ds(pl.multiple_of((p // 16) * 16, 16), 16), :].astype(f32)
        return jnp.sum(jnp.where(r16 == p % 16, g, 0.0), axis=0, keepdims=True)

    xs = jnp.where(r16 == 0, pick(p0), jnp.where(r16 == 1, pick(p1), 0.0)).astype(bf16)
    for cp in f_cps:
        cp.wait()
    g = _rb(jnp.dot(xs, wg_v[...], preferred_element_type=f32))
    u = _rb(jnp.dot(xs, wu_v[...], preferred_element_type=f32))
    g = _rb(g * jax.nn.sigmoid(g))
    y = _rb(jnp.dot((g * u).astype(bf16), wd_v[...], preferred_element_type=f32))
    rs = jnp.where(r16 == 0, r0, r1)
    y = _rb(y * _rb(jax.nn.sigmoid(rs)))
    y0 = y[0:1, :]
    y1 = y[1:2, :]
    rowt = jax.lax.broadcasted_iota(jnp.int32, (16, 128), 0)

    def phase_b(b, carry):
        base = pl.multiple_of(b * R, R)
        ys = None
        hs = []
        for n in range(G):
            h = carry[n]
            seq = []
            for j in range(J):
                h = step(n, h, bu_v[pl.ds(base + NSEG * j, NSEG), 256 * n:256 * (n + 1)])
                seq.append(jnp.concatenate(h, axis=1))
            hs.append(h)
            cn = slice(128 * n, 128 * (n + 1))
            cw = jnp.concatenate([xn_v[L:L + D, cn], xn_v[L + D:, cn]], axis=1)
            y = jax.lax.dot_general(jnp.concatenate(seq, axis=0).astype(bf16), cw, _NT,
                                    preferred_element_type=f32)
            ys = y if ys is None else ys + y
        for g in range(G):
            cg = slice(128 * g, 128 * (g + 1))
            for q in range(R // 16):
                row = pl.multiple_of(b * R + 16 * q, 16)
                t = ys[16 * q:16 * (q + 1), cg]
                t = t + xn_v[pl.ds(row, 16), cg].astype(f32) * dsk1[:, cg]
                t = jnp.where(rowt == p0 - row, t + y0[:, cg], t)
                t = jnp.where(rowt == p1 - row, t + y1[:, cg], t)
                for j in range(2):
                    st_v[g, pl.ds(PB * (2 * q + j), 8), :] = t[8 * j:8 * (j + 1), :]
            for s in range(NSEG):
                nat = pl.ds(pl.multiple_of(s * SEG + b * J, J), J)
                o_v[nat, cg] = x_v[nat, cg].astype(f32) + st_v[g, pl.ds(s, J, stride=PB), :]
        for s in range(NSEG):
            o_cp(b, s).start()
        return hs

    jax.lax.fori_loop(0, NB, phase_b,
                      [(hr[:, 128 * n:128 * (n + 1)], hi[:, 128 * n:128 * (n + 1)]) for n in range(G)])
    pltpu.make_async_copy(o_v, o_v, so.at[0]).wait()


@jax.jit
def pallas_parallel_sum__ssm_conv_s5__moe_arch_mod__prompt_kernel(
    A_x: jax.Array,
    A_Lambda_re: jax.Array,
    A_Lambda_im: jax.Array,
    A_B_re: jax.Array,
    A_B_im: jax.Array,
    A_C_re: jax.Array,
    A_C_im: jax.Array,
    A_log_dt: jax.Array,
    A_Dskip: jax.Array,
    B_x: jax.Array,
    B_w_r: jax.Array,
    B_w_gate: jax.Array,
    B_w_up: jax.Array,
    B_w_down: jax.Array,
):
    del B_x
    hbm = pl.BlockSpec(memory_space=pl.ANY)
    vec = pl.BlockSpec(memory_space=pltpu.VMEM)
    out = pl.pallas_call(
        _kernel,
        out_shape=jax.ShapeDtypeStruct((L, D), f32),
        in_specs=[hbm, vec, vec, hbm, hbm, hbm, hbm, vec, vec, vec, hbm, hbm, hbm],
        out_specs=hbm,
        scratch_shapes=[
            pltpu.VMEM((L, D), bf16),
            pltpu.VMEM((L + 2 * D, D), bf16),
            pltpu.VMEM((2 * P, D), bf16),
            pltpu.VMEM((2, D, P), bf16),
            pltpu.VMEM((L, 2 * P), f32),
            pltpu.VMEM((L, D), f32),
            pltpu.VMEM((G, PB * J, 128), f32),
            pltpu.VMEM((D, F), bf16),
            pltpu.VMEM((D, F), bf16),
            pltpu.VMEM((F, D), bf16),
            pltpu.SemaphoreType.DMA((NB,)),
            pltpu.SemaphoreType.DMA((NA,)),
            pltpu.SemaphoreType.DMA((7,)),
            pltpu.SemaphoreType.DMA((1,)),
        ],
        compiler_params=pltpu.CompilerParams(vmem_limit_bytes=100 * 1024 * 1024),
    )(
        A_x.reshape(L, D),
        A_Lambda_re, A_Lambda_im,
        A_B_re, A_B_im, A_C_re, A_C_im,
        A_log_dt, A_Dskip, B_w_r,
        B_w_gate, B_w_up, B_w_down,
    )
    return out.reshape(1, L, D)
```

```python
import jax
import jax.numpy as jnp
import numpy as np
import jax.experimental.pallas as pl
import jax.experimental.pallas.tpu as pltpu

L = 2048
D = 1024
P = 1024
F = 3584
NSEG = 8
SEG = L // NSEG
J = 32
NB = SEG // J
R = NSEG * J
G = D // 128
NA = 8
AHEAD = 3
PA = J + 4
PB = 12

_NT = (((1,), (1,)), ((), ()))
f32 = jnp.float32
bf16 = jnp.bfloat16


def _rb(v):
    return v.astype(bf16).astype(f32)


def _kernel(x_hbm, lre_ref, lim_ref, bre_hbm, bim_hbm, cre_hbm, cim_hbm, ldt_ref,
            dsk_ref, wr_ref, wg_hbm, wu_hbm, wd_hbm, out_hbm,
            x_v, xn_v, b_v, craw_v, bu_v, o_v, st_v, wg_v, wu_v, wd_v,
            sx, sb, sw, so):
    def x_cp(b, s):
        rows = pl.ds(pl.multiple_of(s * SEG + b * J, J), J)
        return pltpu.make_async_copy(x_hbm.at[rows], x_v.at[rows], sx.at[b])

    def b_cp(n):
        return [pltpu.make_async_copy(src.at[pl.ds(n * 128, 128)],
                                      b_v.at[pl.ds(n * 256 + i * 128, 128)], sb.at[n])
                for i, src in enumerate((bre_hbm, bim_hbm))]

    def o_cp(b, s):
        rows = pl.ds(pl.multiple_of(s * SEG + b * J, J), J)
        return pltpu.make_async_copy(o_v.at[rows], out_hbm.at[rows], so.at[0])

    c_cps = [pltpu.make_async_copy(cre_hbm, craw_v.at[0], sw.at[2]),
             pltpu.make_async_copy(cim_hbm, craw_v.at[1], sw.at[3])]
    f_cps = [pltpu.make_async_copy(wg_hbm, wg_v, sw.at[4]),
             pltpu.make_async_copy(wu_hbm, wu_v, sw.at[5]),
             pltpu.make_async_copy(wd_hbm, wd_v, sw.at[6])]

    for b in range(1):
        for s in range(NSEG):
            x_cp(b, s).start()

    dt = _rb(jnp.exp(ldt_ref[...].astype(f32).reshape(1, D)))
    lre = lre_ref[...].astype(f32).reshape(1, D)
    lim = lim_ref[...].astype(f32).reshape(1, D)
    mag = jnp.exp(dt * lre)
    a_re = mag * jnp.cos(dt * lim)
    a_im = mag * jnp.sin(dt * lim)
    den = lre * lre + lim * lim
    k_re = 2.0 * ((a_re - 1.0) * lre + a_im * lim) / den
    k_im = 2.0 * (a_im * lre - (a_re - 1.0) * lim) / den
    ar8 = jnp.broadcast_to(a_re, (NSEG, P))
    ai8 = jnp.broadcast_to(a_im, (NSEG, P))
    wr = wr_ref[...].astype(f32).reshape(1, D)
    eps = f32(np.float32(np.asarray(1e-5, dtype=bf16)))

    dsk1 = dsk_ref[...].astype(f32).reshape(1, D) + 1.0
    lane = jax.lax.broadcasted_iota(jnp.int32, (NSEG, SEG), 1)
    sub = jax.lax.broadcasted_iota(jnp.int32, (NSEG, SEG), 0)

    def tie(v, z):
        return v if z is None else pltpu.bitcast(pltpu.bitcast(v, jnp.int32) | z, f32)

    def norm_rows(b, q, racc, z=None):
        x = jnp.concatenate([
            jnp.concatenate([tie(st_v[g, pl.ds(2 * q + j, NSEG, stride=PA), :], z if g == 0 else None) for g in range(G)], axis=1)
            for j in range(2)], axis=0)
        m = jnp.sum(x, axis=-1, keepdims=True) * (1.0 / D)
        c = x - m
        v = jnp.sum(c * c, axis=-1, keepdims=True) * (1.0 / D)
        sd = _rb(jnp.sqrt(_rb(_rb(v) + eps)))
        xn = (_rb(x - _rb(m)) * (1.0 / sd)).astype(bf16)
        xn_v[pl.ds(pl.multiple_of(b * R + 16 * q, 16), 16), :] = xn
        r = _rb(jnp.sum(xn.astype(f32) * wr, axis=-1, keepdims=True))
        for j in range(2):
            racc = jnp.where(lane == b * J + 2 * q + j, r[NSEG * j:NSEG * (j + 1), :], racc)
        return racc

    def stage(b, s, z=None):
        nat = pl.ds(pl.multiple_of(s * SEG + b * J, J), J)
        for g in range(G):
            zz = None if z is None else jnp.concatenate([z] * (J // 8), axis=0)
            st_v[g, s * PA:s * PA + J, :] = tie(x_v[nat, 128 * g:128 * (g + 1)].astype(f32), zz)

    def step(n, h, bu):
        ar, ai = ar8[:, 128 * n:128 * (n + 1)], ai8[:, 128 * n:128 * (n + 1)]
        return (ar * h[0] - ai * h[1] + bu[:, :128], ar * h[1] + ai * h[0] + bu[:, 128:])

    def in_proj(b, n, h):
        rows = pl.ds(pl.multiple_of(b * R, R), R)
        cols = slice(n * 256, (n + 1) * 256)
        bu = jax.lax.dot_general(xn_v[rows, :], b_v[cols, :], _NT, preferred_element_type=f32)
        bu_v[rows, cols] = bu
        for j in range(J):
            h = step(n, h, bu[NSEG * j:NSEG * (j + 1), :])
        t = pltpu.bitcast(bu[:, :128], jnp.int32)
        zs = [(t[8 * i:8 * i + 8] * t[8 * i:8 * i + 8]) & 2 for i in range(0, J, J // 4)]
        return h, zs

    def cprep(row):
        rows = pl.ds(pl.multiple_of(row, 16), 16)
        cre = craw_v[0, rows, :].astype(f32)
        cim = craw_v[1, rows, :].astype(f32)
        xn_v[pl.ds(pl.multiple_of(L + row, 16), 16), :] = (cre * k_re - cim * k_im).astype(bf16)
        xn_v[pl.ds(pl.multiple_of(L + D + row, 16), 16), :] = (cre * (-k_im) - cim * k_re).astype(bf16)

    z = jnp.zeros((NSEG, 128), f32)
    hs = []
    for n in range(AHEAD):
        for cp in b_cp(n):
            cp.start()
    for s in range(NSEG):
        x_cp(0, s).wait()
        stage(0, s)
    racc = jnp.zeros((NSEG, SEG), f32)
    for q in range(R // 16):
        racc = norm_rows(0, q, racc)

    def phase_a(b, carry, with_c=False, first=False, last=False, second=False):
        hp, racc = carry
        hs = []
        if not last and not first:
            for s in range(NSEG):
                x_cp(b + 1, s).wait()

        for n in range(NA):
            if first:
                for cp in b_cp(n):
                    cp.wait()
                if n + AHEAD < NA:
                    for cp in b_cp(n + AHEAD):
                        cp.start()
                for s in range(NSEG):
                    if n == 1:
                        x_cp(1, s).start()
                    if n == 4:
                        x_cp(1, s).wait()
                    if n == NA - AHEAD:
                        x_cp(2, s).start()
                    if n == NA - 1:
                        for bb in range(3, NB):
                            x_cp(bb, s).start()
            if second and n == NA // 2:
                for cp in c_cps + f_cps:
                    cp.start()
            h, zs = in_proj(b, n, hp[n])
            hs.append(h)
            if not last and not first:
                if n < 2:
                    for i in range(4):
                        stage(b + 1, 4 * n + i, zs[i])
                else:
                    qs = range((n - 2) * 16 // 6, (n - 1) * 16 // 6)
                    for i, q in enumerate(qs):
                        racc = norm_rows(b + 1, q, racc, zs[i])
            if first and n == 4:
                for i in range(8):
                    stage(1, i, zs[i // 2])
            if first and n > 4:
                for i, q in enumerate(range((n - 5) * 16 // 3, (n - 4) * 16 // 3)):
                    racc = norm_rows(1, q, racc, zs[i % 4])
            if with_c:
                k = 2 * D // NB // NA
                for i in range(k // 16):
                    cprep(((b - NB // 2) * NA + n) * k + 16 * i)
        return hs, racc

    hs, racc = phase_a(0, ([(z, z)] * NA, racc), first=True)
    hs = jax.lax.fori_loop(2, NB // 2, phase_a, phase_a(1, (hs, racc), second=True))
    for cp in c_cps:
        cp.wait()
    hs = jax.lax.fori_loop(
        NB // 2, NB - 1, lambda b, c: phase_a(b, c, True), hs)
    hs, racc = phase_a(NB - 1, hs, True, last=True)
    er = jnp.concatenate([h[0] for h in hs], axis=1)
    ei = jnp.concatenate([h[1] for h in hs], axis=1)
    pr, pi = ar8, ai8
    n = 1
    while n < SEG:
        pr, pi = pr * pr - pi * pi, 2.0 * pr * pi
        n *= 2
    srow = jax.lax.broadcasted_iota(jnp.int32, (NSEG, P), 0)
    hr = jnp.where(srow >= 1, pltpu.roll(er, 1, 0), 0.0)
    hi = jnp.where(srow >= 1, pltpu.roll(ei, 1, 0), 0.0)
    for sh in (1, 2, 4):
        tr = jnp.where(srow >= sh, pltpu.roll(hr, sh, 0), 0.0)
        ti = jnp.where(srow >= sh, pltpu.roll(hi, sh, 0), 0.0)
        hr, hi = hr + pr * tr - pi * ti, hi + pr * ti + pi * tr
        pr, pi = pr * pr - pi * pi, 2.0 * pr * pi

    tok = sub * SEG + lane
    r0 = jnp.max(racc)
    i0 = jnp.min(jnp.where(racc == r0, tok, L))
    rest = jnp.where(tok == i0, -jnp.inf, racc)
    r1 = jnp.max(rest)
    i1 = jnp.min(jnp.where((rest == r1) & (tok != i0), tok, L))
    i0 = jnp.clip(i0, 0, L - 1)
    i1 = jnp.clip(i1, 0, L - 1)
    p0 = (i0 % SEG) * NSEG + i0 // SEG
    p1 = (i1 % SEG) * NSEG + i1 // SEG
    r16 = jax.lax.broadcasted_iota(jnp.int32, (16, D), 0)

    def pick(p):
        g = xn_v[pl.ds(pl.multiple_of((p // 16) * 16, 16), 16), :].astype(f32)
        return jnp.sum(jnp.where(r16 == p % 16, g, 0.0), axis=0, keepdims=True)

    xs = jnp.where(r16 == 0, pick(p0), jnp.where(r16 == 1, pick(p1), 0.0)).astype(bf16)
    for cp in f_cps:
        cp.wait()
    g = _rb(jnp.dot(xs, wg_v[...], preferred_element_type=f32))
    u = _rb(jnp.dot(xs, wu_v[...], preferred_element_type=f32))
    g = _rb(g * jax.nn.sigmoid(g))
    y = _rb(jnp.dot((g * u).astype(bf16), wd_v[...], preferred_element_type=f32))
    rs = jnp.where(r16 == 0, r0, r1)
    y = _rb(y * _rb(jax.nn.sigmoid(rs)))
    y0 = y[0:1, :]
    y1 = y[1:2, :]
    rowt = jax.lax.broadcasted_iota(jnp.int32, (16, 128), 0)

    def phase_b(b, carry):
        base = pl.multiple_of(b * R, R)
        ys = None
        hs = []
        for n in range(G):
            h = carry[n]
            seq = []
            for j in range(J):
                h = step(n, h, bu_v[pl.ds(base + NSEG * j, NSEG), 256 * n:256 * (n + 1)])
                seq.append(jnp.concatenate(h, axis=1))
            hs.append(h)
            cn = slice(128 * n, 128 * (n + 1))
            cw = jnp.concatenate([xn_v[L:L + D, cn], xn_v[L + D:, cn]], axis=1)
            y = jax.lax.dot_general(jnp.concatenate(seq, axis=0).astype(bf16), cw, _NT,
                                    preferred_element_type=f32)
            ys = y if ys is None else ys + y
        for g in range(G):
            cg = slice(128 * g, 128 * (g + 1))
            for q in range(R // 16):
                row = pl.multiple_of(b * R + 16 * q, 16)
                t = ys[16 * q:16 * (q + 1), cg]
                t = t + xn_v[pl.ds(row, 16), cg].astype(f32) * dsk1[:, cg]
                t = jnp.where(rowt == p0 - row, t + y0[:, cg], t)
                t = jnp.where(rowt == p1 - row, t + y1[:, cg], t)
                for j in range(2):
                    st_v[g, pl.ds(PB * (2 * q + j), 8), :] = t[8 * j:8 * (j + 1), :]
            for s in range(NSEG):
                nat = pl.ds(pl.multiple_of(s * SEG + b * J, J), J)
                o_v[nat, cg] = x_v[nat, cg].astype(f32) + st_v[g, pl.ds(s, J, stride=PB), :]
        for s in range(NSEG):
            o_cp(b, s).start()
        return hs

    jax.lax.fori_loop(0, NB, phase_b,
                      [(hr[:, 128 * n:128 * (n + 1)], hi[:, 128 * n:128 * (n + 1)]) for n in range(G)])
    pltpu.make_async_copy(o_v, o_v, so.at[0]).wait()


@jax.jit
def pallas_parallel_sum__ssm_conv_s5__moe_arch_mod__prompt_kernel(
    A_x: jax.Array,
    A_Lambda_re: jax.Array,
    A_Lambda_im: jax.Array,
    A_B_re: jax.Array,
    A_B_im: jax.Array,
    A_C_re: jax.Array,
    A_C_im: jax.Array,
    A_log_dt: jax.Array,
    A_Dskip: jax.Array,
    B_x: jax.Array,
    B_w_r: jax.Array,
    B_w_gate: jax.Array,
    B_w_up: jax.Array,
    B_w_down: jax.Array,
):
    del B_x
    hbm = pl.BlockSpec(memory_space=pl.ANY)
    vec = pl.BlockSpec(memory_space=pltpu.VMEM)
    out = pl.pallas_call(
        _kernel,
        out_shape=jax.ShapeDtypeStruct((L, D), f32),
        in_specs=[hbm, vec, vec, hbm, hbm, hbm, hbm, vec, vec, vec, hbm, hbm, hbm],
        out_specs=hbm,
        scratch_shapes=[
            pltpu.VMEM((L, D), bf16),
            pltpu.VMEM((L + 2 * D, D), bf16),
            pltpu.VMEM((2 * P, D), bf16),
            pltpu.VMEM((2, D, P), bf16),
            pltpu.VMEM((L, 2 * P), f32),
            pltpu.VMEM((L, D), f32),
            pltpu.VMEM((G, PB * J, 128), f32),
            pltpu.VMEM((D, F), bf16),
            pltpu.VMEM((D, F), bf16),
            pltpu.VMEM((F, D), bf16),
            pltpu.SemaphoreType.DMA((NB,)),
            pltpu.SemaphoreType.DMA((NA,)),
            pltpu.SemaphoreType.DMA((7,)),
            pltpu.SemaphoreType.DMA((1,)),
        ],
        compiler_params=pltpu.CompilerParams(vmem_limit_bytes=100 * 1024 * 1024),
    )(
        A_x.reshape(L, D),
        A_Lambda_re, A_Lambda_im,
        A_B_re, A_B_im, A_C_re, A_C_im,
        A_log_dt, A_Dskip, B_w_r,
        B_w_gate, B_w_up, B_w_down,
    )
    return out.reshape(1, L, D)
```

```python
import jax
import jax.numpy as jnp
import numpy as np
import jax.experimental.pallas as pl
import jax.experimental.pallas.tpu as pltpu

L = 2048
D = 1024
P = 1024
F = 3584
NSEG = 8
SEG = L // NSEG
J = 32
NB = SEG // J
R = NSEG * J
G = D // 128
NA = 8
AHEAD = 3
PA = J + 4
PB = 12

_NT = (((1,), (1,)), ((), ()))
f32 = jnp.float32
bf16 = jnp.bfloat16


def _rb(v):
    return v.astype(bf16).astype(f32)


def _kernel(x_hbm, lre_ref, lim_ref, bre_hbm, bim_hbm, cre_hbm, cim_hbm, ldt_ref,
            dsk_ref, wr_ref, wg_hbm, wu_hbm, wd_hbm, out_hbm,
            x_v, xn_v, b_v, craw_v, bu_v, o_v, st_v, wg_v, wu_v, wd_v,
            sx, sb, sw, so):
    def x_cp(b, s):
        rows = pl.ds(pl.multiple_of(s * SEG + b * J, J), J)
        return pltpu.make_async_copy(x_hbm.at[rows], x_v.at[rows], sx.at[b])

    def b_cp(n):
        return [pltpu.make_async_copy(src.at[pl.ds(n * 128, 128)],
                                      b_v.at[pl.ds(n * 256 + i * 128, 128)], sb.at[n])
                for i, src in enumerate((bre_hbm, bim_hbm))]

    def o_cp(b, s):
        rows = pl.ds(pl.multiple_of(s * SEG + b * J, J), J)
        return pltpu.make_async_copy(o_v.at[rows], out_hbm.at[rows], so.at[0])

    c_cps = [pltpu.make_async_copy(cre_hbm, craw_v.at[0], sw.at[2]),
             pltpu.make_async_copy(cim_hbm, craw_v.at[1], sw.at[3])]
    f_cps = [pltpu.make_async_copy(wg_hbm, wg_v, sw.at[4]),
             pltpu.make_async_copy(wu_hbm, wu_v, sw.at[5]),
             pltpu.make_async_copy(wd_hbm, wd_v, sw.at[6])]

    for b in range(1):
        for s in range(NSEG):
            x_cp(b, s).start()

    dt = _rb(jnp.exp(ldt_ref[...].astype(f32).reshape(1, D)))
    lre = lre_ref[...].astype(f32).reshape(1, D)
    lim = lim_ref[...].astype(f32).reshape(1, D)
    mag = jnp.exp(dt * lre)
    a_re = mag * jnp.cos(dt * lim)
    a_im = mag * jnp.sin(dt * lim)
    den = lre * lre + lim * lim
    k_re = 2.0 * ((a_re - 1.0) * lre + a_im * lim) / den
    k_im = 2.0 * (a_im * lre - (a_re - 1.0) * lim) / den
    ar8 = jnp.broadcast_to(a_re, (NSEG, P))
    ai8 = jnp.broadcast_to(a_im, (NSEG, P))
    wr = wr_ref[...].astype(f32).reshape(1, D)
    eps = f32(np.float32(np.asarray(1e-5, dtype=bf16)))

    dsk1 = dsk_ref[...].astype(f32).reshape(1, D) + 1.0
    lane = jax.lax.broadcasted_iota(jnp.int32, (NSEG, SEG), 1)
    sub = jax.lax.broadcasted_iota(jnp.int32, (NSEG, SEG), 0)

    def tie(v, z):
        return v if z is None else pltpu.bitcast(pltpu.bitcast(v, jnp.int32) | z, f32)

    def norm_rows(b, q, racc, z=None):
        x = jnp.concatenate([
            jnp.concatenate([tie(st_v[g, pl.ds(2 * q + j, NSEG, stride=PA), :], z if g == 0 else None) for g in range(G)], axis=1)
            for j in range(2)], axis=0)
        m = jnp.sum(x, axis=-1, keepdims=True) * (1.0 / D)
        c = x - m
        v = jnp.sum(c * c, axis=-1, keepdims=True) * (1.0 / D)
        sd = _rb(jnp.sqrt(_rb(_rb(v) + eps)))
        xn = (_rb(x - _rb(m)) * (1.0 / sd)).astype(bf16)
        xn_v[pl.ds(pl.multiple_of(b * R + 16 * q, 16), 16), :] = xn
        r = _rb(jnp.sum(xn.astype(f32) * wr, axis=-1, keepdims=True))
        for j in range(2):
            racc = jnp.where(lane == b * J + 2 * q + j, r[NSEG * j:NSEG * (j + 1), :], racc)
        return racc

    def stage(b, s, z=None):
        nat = pl.ds(pl.multiple_of(s * SEG + b * J, J), J)
        for g in range(G):
            zz = None if z is None else jnp.concatenate([z] * (J // 8), axis=0)
            st_v[g, s * PA:s * PA + J, :] = tie(x_v[nat, 128 * g:128 * (g + 1)].astype(f32), zz)

    def step(n, h, bu):
        ar, ai = ar8[:, 128 * n:128 * (n + 1)], ai8[:, 128 * n:128 * (n + 1)]
        return (ar * h[0] - ai * h[1] + bu[:, :128], ar * h[1] + ai * h[0] + bu[:, 128:])

    def in_proj(b, n, h):
        rows = pl.ds(pl.multiple_of(b * R, R), R)
        cols = slice(n * 256, (n + 1) * 256)
        bu = jax.lax.dot_general(xn_v[rows, :], b_v[cols, :], _NT, preferred_element_type=f32)
        bu_v[rows, cols] = bu
        for j in range(J):
            h = step(n, h, bu[NSEG * j:NSEG * (j + 1), :])
        t = pltpu.bitcast(bu[:, :128], jnp.int32)
        zs = [(t[8 * i:8 * i + 8] * t[8 * i:8 * i + 8]) & 2 for i in range(0, J, J // 4)]
        return h, zs

    def cprep(row, z):
        rows = pl.ds(pl.multiple_of(row, 16), 16)
        zz = jnp.concatenate([jnp.concatenate([z, z], axis=0)] * G, axis=1)
        cre = tie(craw_v[0, rows, :].astype(f32), zz)
        cim = craw_v[1, rows, :].astype(f32)
        xn_v[pl.ds(pl.multiple_of(L + row, 16), 16), :] = (cre * k_re - cim * k_im).astype(bf16)
        xn_v[pl.ds(pl.multiple_of(L + D + row, 16), 16), :] = (cre * (-k_im) - cim * k_re).astype(bf16)

    z = jnp.zeros((NSEG, 128), f32)
    hs = []
    for n in range(AHEAD):
        for cp in b_cp(n):
            cp.start()
    for s in range(NSEG):
        x_cp(0, s).wait()
    for s in range(NSEG):
        stage(0, s)
    racc = jnp.zeros((NSEG, SEG), f32)
    for q in range(R // 16):
        racc = norm_rows(0, q, racc)

    def phase_a(b, carry, with_c=False, first=False, last=False, second=False):
        hp, racc = carry
        hs = []
        if not last and not first:
            for s in range(NSEG):
                x_cp(b + 1, s).wait()

        for n in range(NA):
            if first:
                for cp in b_cp(n):
                    cp.wait()
                if n + AHEAD < NA:
                    for cp in b_cp(n + AHEAD):
                        cp.start()
                for s in range(NSEG):
                    if n == 1:
                        x_cp(1, s).start()
                    if n == 4:
                        x_cp(1, s).wait()
                    if n == NA - AHEAD:
                        x_cp(2, s).start()
                    if n == NA - 1:
                        for bb in range(3, NB):
                            x_cp(bb, s).start()
            if second and n == NA // 2:
                for cp in c_cps + f_cps:
                    cp.start()
            h, zs = in_proj(b, n, hp[n])
            hs.append(h)
            if not last and not first:
                if n < 2:
                    for i in range(4):
                        stage(b + 1, 4 * n + i, zs[i])
                else:
                    qs = range((n - 2) * 16 // 6, (n - 1) * 16 // 6)
                    for i, q in enumerate(qs):
                        racc = norm_rows(b + 1, q, racc, zs[i])
            if first and n == 4:
                for i in range(8):
                    stage(1, i, zs[i // 2])
            if first and n > 4:
                for i, q in enumerate(range((n - 5) * 16 // 3, (n - 4) * 16 // 3)):
                    racc = norm_rows(1, q, racc, zs[i % 4])
            if with_c:
                k = 2 * D // NB // NA
                for i in range(k // 16):
                    cprep(((b - NB // 2) * NA + n) * k + 16 * i, zs[2 * i + 1])
        return hs, racc

    hs, racc = phase_a(0, ([(z, z)] * NA, racc), first=True)
    hs = jax.lax.fori_loop(2, NB // 2, phase_a, phase_a(1, (hs, racc), second=True))
    for cp in c_cps:
        cp.wait()
    hs = jax.lax.fori_loop(
        NB // 2, NB - 1, lambda b, c: phase_a(b, c, True), hs)
    hs, racc = phase_a(NB - 1, hs, True, last=True)
    er = jnp.concatenate([h[0] for h in hs], axis=1)
    ei = jnp.concatenate([h[1] for h in hs], axis=1)
    pr, pi = ar8, ai8
    n = 1
    while n < SEG:
        pr, pi = pr * pr - pi * pi, 2.0 * pr * pi
        n *= 2
    srow = jax.lax.broadcasted_iota(jnp.int32, (NSEG, P), 0)
    hr = jnp.where(srow >= 1, pltpu.roll(er, 1, 0), 0.0)
    hi = jnp.where(srow >= 1, pltpu.roll(ei, 1, 0), 0.0)
    for sh in (1, 2, 4):
        tr = jnp.where(srow >= sh, pltpu.roll(hr, sh, 0), 0.0)
        ti = jnp.where(srow >= sh, pltpu.roll(hi, sh, 0), 0.0)
        hr, hi = hr + pr * tr - pi * ti, hi + pr * ti + pi * tr
        pr, pi = pr * pr - pi * pi, 2.0 * pr * pi

    tok = sub * SEG + lane
    r0 = jnp.max(racc)
    i0 = jnp.min(jnp.where(racc == r0, tok, L))
    rest = jnp.where(tok == i0, -jnp.inf, racc)
    r1 = jnp.max(rest)
    i1 = jnp.min(jnp.where((rest == r1) & (tok != i0), tok, L))
    i0 = jnp.clip(i0, 0, L - 1)
    i1 = jnp.clip(i1, 0, L - 1)
    p0 = (i0 % SEG) * NSEG + i0 // SEG
    p1 = (i1 % SEG) * NSEG + i1 // SEG
    r16 = jax.lax.broadcasted_iota(jnp.int32, (16, D), 0)

    def pick(p):
        g = xn_v[pl.ds(pl.multiple_of((p // 16) * 16, 16), 16), :].astype(f32)
        return jnp.sum(jnp.where(r16 == p % 16, g, 0.0), axis=0, keepdims=True)

    xs = jnp.where(r16 == 0, pick(p0), jnp.where(r16 == 1, pick(p1), 0.0)).astype(bf16)
    for cp in f_cps:
        cp.wait()
    g = _rb(jnp.dot(xs, wg_v[...], preferred_element_type=f32))
    u = _rb(jnp.dot(xs, wu_v[...], preferred_element_type=f32))
    g = _rb(g * jax.nn.sigmoid(g))
    y = _rb(jnp.dot((g * u).astype(bf16), wd_v[...], preferred_element_type=f32))
    rs = jnp.where(r16 == 0, r0, r1)
    y = _rb(y * _rb(jax.nn.sigmoid(rs)))
    y0 = y[0:1, :]
    y1 = y[1:2, :]
    rowt = jax.lax.broadcasted_iota(jnp.int32, (16, 128), 0)

    def phase_b(b, carry):
        base = pl.multiple_of(b * R, R)
        ys = None
        hs = []
        for n in range(G):
            h = carry[n]
            seq = []
            for j in range(J):
                h = step(n, h, bu_v[pl.ds(base + NSEG * j, NSEG), 256 * n:256 * (n + 1)])
                seq.append(jnp.concatenate(h, axis=1))
            hs.append(h)
            cn = slice(128 * n, 128 * (n + 1))
            cw = jnp.concatenate([xn_v[L:L + D, cn], xn_v[L + D:, cn]], axis=1)
            y = jax.lax.dot_general(jnp.concatenate(seq, axis=0).astype(bf16), cw, _NT,
                                    preferred_element_type=f32)
            ys = y if ys is None else ys + y
        for g in range(G):
            cg = slice(128 * g, 128 * (g + 1))
            for q in range(R // 16):
                row = pl.multiple_of(b * R + 16 * q, 16)
                t = ys[16 * q:16 * (q + 1), cg]
                t = t + xn_v[pl.ds(row, 16), cg].astype(f32) * dsk1[:, cg]
                t = jnp.where(rowt == p0 - row, t + y0[:, cg], t)
                t = jnp.where(rowt == p1 - row, t + y1[:, cg], t)
                for j in range(2):
                    st_v[g, pl.ds(PB * (2 * q + j), 8), :] = t[8 * j:8 * (j + 1), :]
            for s in range(NSEG):
                nat = pl.ds(pl.multiple_of(s * SEG + b * J, J), J)
                o_v[nat, cg] = x_v[nat, cg].astype(f32) + st_v[g, pl.ds(s, J, stride=PB), :]
        for s in range(NSEG):
            o_cp(b, s).start()
        return hs

    jax.lax.fori_loop(0, NB, phase_b,
                      [(hr[:, 128 * n:128 * (n + 1)], hi[:, 128 * n:128 * (n + 1)]) for n in range(G)])
    pltpu.make_async_copy(o_v, o_v, so.at[0]).wait()


@jax.jit
def pallas_parallel_sum__ssm_conv_s5__moe_arch_mod__prompt_kernel(
    A_x: jax.Array,
    A_Lambda_re: jax.Array,
    A_Lambda_im: jax.Array,
    A_B_re: jax.Array,
    A_B_im: jax.Array,
    A_C_re: jax.Array,
    A_C_im: jax.Array,
    A_log_dt: jax.Array,
    A_Dskip: jax.Array,
    B_x: jax.Array,
    B_w_r: jax.Array,
    B_w_gate: jax.Array,
    B_w_up: jax.Array,
    B_w_down: jax.Array,
):
    del B_x
    hbm = pl.BlockSpec(memory_space=pl.ANY)
    vec = pl.BlockSpec(memory_space=pltpu.VMEM)
    out = pl.pallas_call(
        _kernel,
        out_shape=jax.ShapeDtypeStruct((L, D), f32),
        in_specs=[hbm, vec, vec, hbm, hbm, hbm, hbm, vec, vec, vec, hbm, hbm, hbm],
        out_specs=hbm,
        scratch_shapes=[
            pltpu.VMEM((L, D), bf16),
            pltpu.VMEM((L + 2 * D, D), bf16),
            pltpu.VMEM((2 * P, D), bf16),
            pltpu.VMEM((2, D, P), bf16),
            pltpu.VMEM((L, 2 * P), f32),
            pltpu.VMEM((L, D), f32),
            pltpu.VMEM((G, PB * J, 128), f32),
            pltpu.VMEM((D, F), bf16),
            pltpu.VMEM((D, F), bf16),
            pltpu.VMEM((F, D), bf16),
            pltpu.SemaphoreType.DMA((NB,)),
            pltpu.SemaphoreType.DMA((NA,)),
            pltpu.SemaphoreType.DMA((7,)),
            pltpu.SemaphoreType.DMA((1,)),
        ],
        compiler_params=pltpu.CompilerParams(vmem_limit_bytes=100 * 1024 * 1024),
    )(
        A_x.reshape(L, D),
        A_Lambda_re, A_Lambda_im,
        A_B_re, A_B_im, A_C_re, A_C_im,
        A_log_dt, A_Dskip, B_w_r,
        B_w_gate, B_w_up, B_w_down,
    )
    return out.reshape(1, L, D)
```

```python
import jax
import jax.numpy as jnp
import numpy as np
import jax.experimental.pallas as pl
import jax.experimental.pallas.tpu as pltpu

L = 2048
D = 1024
P = 1024
F = 3584
NSEG = 8
SEG = L // NSEG
J = 32
NB = SEG // J
R = NSEG * J
G = D // 128
NA = 8
AHEAD = 3
PA = J + 4
PB = 12

_NT = (((1,), (1,)), ((), ()))
f32 = jnp.float32
bf16 = jnp.bfloat16


def _rb(v):
    return v.astype(bf16).astype(f32)


def _kernel(x_hbm, lre_ref, lim_ref, bre_hbm, bim_hbm, cre_hbm, cim_hbm, ldt_ref,
            dsk_ref, wr_ref, wg_hbm, wu_hbm, wd_hbm, out_hbm,
            x_v, xn_v, b_v, craw_v, bu_v, h_v, o_v, st_v, wg_v, wu_v, wd_v,
            sx, sb, sw, so):
    def x_cp(b, s):
        rows = pl.ds(pl.multiple_of(s * SEG + b * J, J), J)
        return pltpu.make_async_copy(x_hbm.at[rows], x_v.at[rows], sx.at[b])

    def b_cp(n):
        return [pltpu.make_async_copy(src.at[pl.ds(n * 128, 128)],
                                      b_v.at[pl.ds(n * 256 + i * 128, 128)], sb.at[n])
                for i, src in enumerate((bre_hbm, bim_hbm))]

    def o_cp(b, s):
        rows = pl.ds(pl.multiple_of(s * SEG + b * J, J), J)
        return pltpu.make_async_copy(o_v.at[rows], out_hbm.at[rows], so.at[0])

    c_cps = [pltpu.make_async_copy(cre_hbm, craw_v.at[0], sw.at[2]),
             pltpu.make_async_copy(cim_hbm, craw_v.at[1], sw.at[3])]
    f_cps = [pltpu.make_async_copy(wg_hbm, wg_v, sw.at[4]),
             pltpu.make_async_copy(wu_hbm, wu_v, sw.at[5]),
             pltpu.make_async_copy(wd_hbm, wd_v, sw.at[6])]

    for b in range(1):
        for s in range(NSEG):
            x_cp(b, s).start()

    dt = _rb(jnp.exp(ldt_ref[...].astype(f32).reshape(1, D)))
    lre = lre_ref[...].astype(f32).reshape(1, D)
    lim = lim_ref[...].astype(f32).reshape(1, D)
    mag = jnp.exp(dt * lre)
    a_re = mag * jnp.cos(dt * lim)
    a_im = mag * jnp.sin(dt * lim)
    den = lre * lre + lim * lim
    k_re = 2.0 * ((a_re - 1.0) * lre + a_im * lim) / den
    k_im = 2.0 * (a_im * lre - (a_re - 1.0) * lim) / den
    ar8 = jnp.broadcast_to(a_re, (NSEG, P))
    ai8 = jnp.broadcast_to(a_im, (NSEG, P))
    wr = wr_ref[...].astype(f32).reshape(1, D)
    eps = f32(np.float32(np.asarray(1e-5, dtype=bf16)))

    dsk1 = dsk_ref[...].astype(f32).reshape(1, D) + 1.0
    lane = jax.lax.broadcasted_iota(jnp.int32, (NSEG, SEG), 1)
    sub = jax.lax.broadcasted_iota(jnp.int32, (NSEG, SEG), 0)

    def tie(v, z):
        return v if z is None else pltpu.bitcast(pltpu.bitcast(v, jnp.int32) | z, f32)

    def norm_rows(b, q, racc, z=None):
        x = jnp.concatenate([
            jnp.concatenate([tie(st_v[g, pl.ds(2 * q + j, NSEG, stride=PA), :], z if g == 0 else None) for g in range(G)], axis=1)
            for j in range(2)], axis=0)
        m = jnp.sum(x, axis=-1, keepdims=True) * (1.0 / D)
        c = x - m
        v = jnp.sum(c * c, axis=-1, keepdims=True) * (1.0 / D)
        sd = _rb(jnp.sqrt(_rb(_rb(v) + eps)))
        xn = (_rb(x - _rb(m)) * (1.0 / sd)).astype(bf16)
        xn_v[pl.ds(pl.multiple_of(b * R + 16 * q, 16), 16), :] = xn
        r = _rb(jnp.sum(xn.astype(f32) * wr, axis=-1, keepdims=True))
        for j in range(2):
            racc = jnp.where(lane == b * J + 2 * q + j, r[NSEG * j:NSEG * (j + 1), :], racc)
        return racc

    def stage(b, s, z=None):
        nat = pl.ds(pl.multiple_of(s * SEG + b * J, J), J)
        for g in range(G):
            zz = None if z is None else jnp.concatenate([z] * (J // 8), axis=0)
            st_v[g, s * PA:s * PA + J, :] = tie(x_v[nat, 128 * g:128 * (g + 1)].astype(f32), zz)

    def step(n, h, bu):
        ar, ai = ar8[:, 128 * n:128 * (n + 1)], ai8[:, 128 * n:128 * (n + 1)]
        return (ar * h[0] - ai * h[1] + bu[:, :128], ar * h[1] + ai * h[0] + bu[:, 128:])

    def in_proj(b, n, h):
        rows = pl.ds(pl.multiple_of(b * R, R), R)
        cols = slice(n * 256, (n + 1) * 256)
        bu = jax.lax.dot_general(xn_v[rows, :], b_v[cols, :], _NT, preferred_element_type=f32)
        bu_v[rows, cols] = bu
        for j in range(J):
            h = step(n, h, bu[NSEG * j:NSEG * (j + 1), :])
        t = pltpu.bitcast(bu[:, :128], jnp.int32)
        zs = [(t[8 * i:8 * i + 8] * t[8 * i:8 * i + 8]) & 2 for i in range(0, J, J // 4)]
        return h, zs

    def cprep(row, z):
        rows = pl.ds(pl.multiple_of(row, 16), 16)
        zz = jnp.concatenate([jnp.concatenate([z, z], axis=0)] * G, axis=1)
        cre = tie(craw_v[0, rows, :].astype(f32), zz)
        cim = craw_v[1, rows, :].astype(f32)
        xn_v[pl.ds(pl.multiple_of(L + row, 16), 16), :] = (cre * k_re - cim * k_im).astype(bf16)
        xn_v[pl.ds(pl.multiple_of(L + D + row, 16), 16), :] = (cre * (-k_im) - cim * k_re).astype(bf16)

    z = jnp.zeros((NSEG, 128), f32)
    hs = []
    for n in range(AHEAD):
        for cp in b_cp(n):
            cp.start()
    for s in range(NSEG):
        x_cp(0, s).wait()
    for s in range(NSEG):
        stage(0, s)
    racc = jnp.zeros((NSEG, SEG), f32)
    for q in range(R // 16):
        racc = norm_rows(0, q, racc)

    def phase_a(b, carry, with_c=False, first=False, last=False, second=False):
        hp, racc = carry
        hs = []
        if not last and not first:
            for s in range(NSEG):
                x_cp(b + 1, s).wait()

        for n in range(NA):
            if first:
                for cp in b_cp(n):
                    cp.wait()
                if n + AHEAD < NA:
                    for cp in b_cp(n + AHEAD):
                        cp.start()
                for s in range(NSEG):
                    if n == 1:
                        x_cp(1, s).start()
                    if n == 4:
                        x_cp(1, s).wait()
                    if n == NA - AHEAD:
                        x_cp(2, s).start()
                    if n == NA - 1:
                        for bb in range(3, NB):
                            x_cp(bb, s).start()
            if second and n == NA // 2:
                for cp in c_cps + f_cps:
                    cp.start()
            h, zs = in_proj(b, n, hp[n])
            hs.append(h)
            if not last and not first:
                if n < 2:
                    for i in range(4):
                        stage(b + 1, 4 * n + i, zs[i])
                else:
                    qs = range((n - 2) * 16 // 6, (n - 1) * 16 // 6)
                    for i, q in enumerate(qs):
                        racc = norm_rows(b + 1, q, racc, zs[i])
            if first and n == 4:
                for i in range(8):
                    stage(1, i, zs[i // 2])
            if first and n > 4:
                for i, q in enumerate(range((n - 5) * 16 // 3, (n - 4) * 16 // 3)):
                    racc = norm_rows(1, q, racc, zs[i % 4])
            if with_c:
                k = 2 * D // NB // NA
                for i in range(k // 16):
                    cprep(((b - NB // 2) * NA + n) * k + 16 * i, zs[2 * i + 1])
        return hs, racc

    hs, racc = phase_a(0, ([(z, z)] * NA, racc), first=True)
    hs = jax.lax.fori_loop(2, NB // 2, phase_a, phase_a(1, (hs, racc), second=True))
    for cp in c_cps:
        cp.wait()
    hs = jax.lax.fori_loop(
        NB // 2, NB - 1, lambda b, c: phase_a(b, c, True), hs)
    hs, racc = phase_a(NB - 1, hs, True, last=True)
    er = jnp.concatenate([h[0] for h in hs], axis=1)
    ei = jnp.concatenate([h[1] for h in hs], axis=1)
    pr, pi = ar8, ai8
    n = 1
    while n < SEG:
        pr, pi = pr * pr - pi * pi, 2.0 * pr * pi
        n *= 2
    srow = jax.lax.broadcasted_iota(jnp.int32, (NSEG, P), 0)
    hr = jnp.where(srow >= 1, pltpu.roll(er, 1, 0), 0.0)
    hi = jnp.where(srow >= 1, pltpu.roll(ei, 1, 0), 0.0)
    for sh in (1, 2, 4):
        tr = jnp.where(srow >= sh, pltpu.roll(hr, sh, 0), 0.0)
        ti = jnp.where(srow >= sh, pltpu.roll(hi, sh, 0), 0.0)
        hr, hi = hr + pr * tr - pi * ti, hi + pr * ti + pi * tr
        pr, pi = pr * pr - pi * pi, 2.0 * pr * pi

    tok = sub * SEG + lane
    r0 = jnp.max(racc)
    i0 = jnp.min(jnp.where(racc == r0, tok, L))
    rest = jnp.where(tok == i0, -jnp.inf, racc)
    r1 = jnp.max(rest)
    i1 = jnp.min(jnp.where((rest == r1) & (tok != i0), tok, L))
    i0 = jnp.clip(i0, 0, L - 1)
    i1 = jnp.clip(i1, 0, L - 1)
    p0 = (i0 % SEG) * NSEG + i0 // SEG
    p1 = (i1 % SEG) * NSEG + i1 // SEG
    r16 = jax.lax.broadcasted_iota(jnp.int32, (16, D), 0)

    def pick(p):
        g = xn_v[pl.ds(pl.multiple_of((p // 16) * 16, 16), 16), :].astype(f32)
        return jnp.sum(jnp.where(r16 == p % 16, g, 0.0), axis=0, keepdims=True)

    xs = jnp.where(r16 == 0, pick(p0), jnp.where(r16 == 1, pick(p1), 0.0)).astype(bf16)
    for cp in f_cps:
        cp.wait()
    g = _rb(jnp.dot(xs, wg_v[...], preferred_element_type=f32))
    u = _rb(jnp.dot(xs, wu_v[...], preferred_element_type=f32))
    g = _rb(g * jax.nn.sigmoid(g))
    y = _rb(jnp.dot((g * u).astype(bf16), wd_v[...], preferred_element_type=f32))
    rs = jnp.where(r16 == 0, r0, r1)
    y = _rb(y * _rb(jax.nn.sigmoid(rs)))
    y0 = y[0:1, :]
    y1 = y[1:2, :]
    rowt = jax.lax.broadcasted_iota(jnp.int32, (16, 128), 0)

    def states(b, n, h, z=None):
        base = pl.multiple_of(b * R, R)
        h = (tie(h[0], z), h[1])
        seq = []
        for j in range(J):
            h = step(n, h, bu_v[pl.ds(base + NSEG * j, NSEG), 256 * n:256 * (n + 1)])
            seq.append(jnp.concatenate(h, axis=1))
        return h, jnp.concatenate(seq, axis=0).astype(bf16)

    def unpermute(b, g, z=None):
        cg = slice(128 * g, 128 * (g + 1))
        zz = None if z is None else jnp.concatenate([z] * (J // 8), axis=0)
        for s in range(NSEG):
            nat = pl.ds(pl.multiple_of(s * SEG + b * J, J), J)
            o_v[nat, cg] = x_v[nat, cg].astype(f32) + tie(st_v[g, pl.ds(s, J, stride=PB), :], zz)

    def phase_b(b, carry, first=False, last=False):
        ys = None
        hs = list(carry)
        for n in range(G):
            if n == 0:
                hq = h_v[...]
            else:
                hs[n], hq = states(b, n, carry[n])
            cn = slice(128 * n, 128 * (n + 1))
            cw = jnp.concatenate([xn_v[L:L + D, cn], xn_v[L + D:, cn]], axis=1)
            y = jax.lax.dot_general(hq, cw, _NT, preferred_element_type=f32)
            ys = y if ys is None else ys + y
            zs = []
            for i in range(2):
                t = pltpu.bitcast(y[:8, 512 * i:512 * i + 128], jnp.int32)
                zs.append((t * t) & 2)
            if not first and n < 4:
                for i in range(2):
                    unpermute(b - 1, 2 * n + i, zs[i])
            if not last and n == G - 2:
                hs[0], hq0 = states(b + 1, 0, carry[0], zs[0])
                h_v[...] = hq0
        if not first:
            for s in range(NSEG):
                o_cp(b - 1, s).start()
        for g in range(G):
            cg = slice(128 * g, 128 * (g + 1))
            for q in range(R // 16):
                row = pl.multiple_of(b * R + 16 * q, 16)
                t = ys[16 * q:16 * (q + 1), cg]
                t = t + xn_v[pl.ds(row, 16), cg].astype(f32) * dsk1[:, cg]
                t = jnp.where(rowt == p0 - row, t + y0[:, cg], t)
                t = jnp.where(rowt == p1 - row, t + y1[:, cg], t)
                for j in range(2):
                    st_v[g, pl.ds(PB * (2 * q + j), 8), :] = t[8 * j:8 * (j + 1), :]
        return hs

    hs = [(hr[:, 128 * n:128 * (n + 1)], hi[:, 128 * n:128 * (n + 1)]) for n in range(G)]
    hs[0], hq = states(0, 0, hs[0])
    h_v[...] = hq
    hs = phase_b(0, hs, first=True)
    hs = jax.lax.fori_loop(1, NB - 1, phase_b, hs)
    phase_b(NB - 1, hs, last=True)
    for g in range(G):
        unpermute(NB - 1, g)
    for s in range(NSEG):
        o_cp(NB - 1, s).start()
    pltpu.make_async_copy(o_v, o_v, so.at[0]).wait()


@jax.jit
def pallas_parallel_sum__ssm_conv_s5__moe_arch_mod__prompt_kernel(
    A_x: jax.Array,
    A_Lambda_re: jax.Array,
    A_Lambda_im: jax.Array,
    A_B_re: jax.Array,
    A_B_im: jax.Array,
    A_C_re: jax.Array,
    A_C_im: jax.Array,
    A_log_dt: jax.Array,
    A_Dskip: jax.Array,
    B_x: jax.Array,
    B_w_r: jax.Array,
    B_w_gate: jax.Array,
    B_w_up: jax.Array,
    B_w_down: jax.Array,
):
    del B_x
    hbm = pl.BlockSpec(memory_space=pl.ANY)
    vec = pl.BlockSpec(memory_space=pltpu.VMEM)
    out = pl.pallas_call(
        _kernel,
        out_shape=jax.ShapeDtypeStruct((L, D), f32),
        in_specs=[hbm, vec, vec, hbm, hbm, hbm, hbm, vec, vec, vec, hbm, hbm, hbm],
        out_specs=hbm,
        scratch_shapes=[
            pltpu.VMEM((L, D), bf16),
            pltpu.VMEM((L + 2 * D, D), bf16),
            pltpu.VMEM((2 * P, D), bf16),
            pltpu.VMEM((2, D, P), bf16),
            pltpu.VMEM((L, 2 * P), f32),
            pltpu.VMEM((R, 256), bf16),
            pltpu.VMEM((L, D), f32),
            pltpu.VMEM((G, PB * J, 128), f32),
            pltpu.VMEM((D, F), bf16),
            pltpu.VMEM((D, F), bf16),
            pltpu.VMEM((F, D), bf16),
            pltpu.SemaphoreType.DMA((NB,)),
            pltpu.SemaphoreType.DMA((NA,)),
            pltpu.SemaphoreType.DMA((7,)),
            pltpu.SemaphoreType.DMA((1,)),
        ],
        compiler_params=pltpu.CompilerParams(vmem_limit_bytes=100 * 1024 * 1024),
    )(
        A_x.reshape(L, D),
        A_Lambda_re, A_Lambda_im,
        A_B_re, A_B_im, A_C_re, A_C_im,
        A_log_dt, A_Dskip, B_w_r,
        B_w_gate, B_w_up, B_w_down,
    )
    return out.reshape(1, L, D)
```

```python
import jax
import jax.numpy as jnp
import numpy as np
import jax.experimental.pallas as pl
import jax.experimental.pallas.tpu as pltpu

L = 2048
D = 1024
P = 1024
F = 3584
NSEG = 8
SEG = L // NSEG
J = 32
NB = SEG // J
R = NSEG * J
G = D // 128
NA = 8
PLAN = {0: ([('b', 0), ('b', 1)], [('b', 2), ('b', 3), ('x', 1), ('b', 4), ('b', 5)]), 2: ([('b', 2), ('b', 3)], [('b', 6), ('b', 7)]), 4: ([('b', 4), ('b', 5), ('x', 1)], [('x', 2)]), 6: ([('b', 6), ('b', 7)], [('x', 3), ('x', 4), ('x', 5), ('x', 6), ('x', 7)])}
AHEAD = 2
PA = J + 4
PB = 12

_NT = (((1,), (1,)), ((), ()))
f32 = jnp.float32
bf16 = jnp.bfloat16


def _rb(v):
    return v.astype(bf16).astype(f32)


def _kernel(x_hbm, lre_ref, lim_ref, bre_hbm, bim_hbm, cre_hbm, cim_hbm, ldt_ref,
            dsk_ref, wr_ref, wg_hbm, wu_hbm, wd_hbm, out_hbm,
            x_v, xn_v, b_v, craw_v, bu_v, h_v, o_v, st_v, wg_v, wu_v, wd_v,
            sx, sb, sw, so):
    def x_cp(b, s):
        rows = pl.ds(pl.multiple_of(s * SEG + b * J, J), J)
        return pltpu.make_async_copy(x_hbm.at[rows], x_v.at[rows], sx.at[b])

    def b_cp(n):
        return [pltpu.make_async_copy(src.at[pl.ds(n * 128, 128)],
                                      b_v.at[pl.ds(n * 256 + i * 128, 128)], sb.at[n])
                for i, src in enumerate((bre_hbm, bim_hbm))]

    def o_cp(b, s):
        rows = pl.ds(pl.multiple_of(s * SEG + b * J, J), J)
        return pltpu.make_async_copy(o_v.at[rows], out_hbm.at[rows], so.at[0])

    c_cps = [pltpu.make_async_copy(cre_hbm, craw_v.at[0], sw.at[2]),
             pltpu.make_async_copy(cim_hbm, craw_v.at[1], sw.at[3])]
    f_cps = [pltpu.make_async_copy(wg_hbm, wg_v, sw.at[4]),
             pltpu.make_async_copy(wu_hbm, wu_v, sw.at[5]),
             pltpu.make_async_copy(wd_hbm, wd_v, sw.at[6])]

    for b in range(1):
        for s in range(NSEG):
            x_cp(b, s).start()

    dt = _rb(jnp.exp(ldt_ref[...].astype(f32).reshape(1, D)))
    lre = lre_ref[...].astype(f32).reshape(1, D)
    lim = lim_ref[...].astype(f32).reshape(1, D)
    mag = jnp.exp(dt * lre)
    a_re = mag * jnp.cos(dt * lim)
    a_im = mag * jnp.sin(dt * lim)
    den = lre * lre + lim * lim
    k_re = 2.0 * ((a_re - 1.0) * lre + a_im * lim) / den
    k_im = 2.0 * (a_im * lre - (a_re - 1.0) * lim) / den
    ar8 = jnp.broadcast_to(a_re, (NSEG, P))
    ai8 = jnp.broadcast_to(a_im, (NSEG, P))
    wr = wr_ref[...].astype(f32).reshape(1, D)
    eps = f32(np.float32(np.asarray(1e-5, dtype=bf16)))

    dsk1 = dsk_ref[...].astype(f32).reshape(1, D) + 1.0
    lane = jax.lax.broadcasted_iota(jnp.int32, (NSEG, SEG), 1)
    sub = jax.lax.broadcasted_iota(jnp.int32, (NSEG, SEG), 0)

    def tie(v, z):
        return v if z is None else pltpu.bitcast(pltpu.bitcast(v, jnp.int32) | z, f32)

    def norm_rows(b, q, racc, z=None):
        x = jnp.concatenate([
            jnp.concatenate([tie(st_v[g, pl.ds(2 * q + j, NSEG, stride=PA), :], z if g == 0 else None) for g in range(G)], axis=1)
            for j in range(2)], axis=0)
        m = jnp.sum(x, axis=-1, keepdims=True) * (1.0 / D)
        c = x - m
        v = jnp.sum(c * c, axis=-1, keepdims=True) * (1.0 / D)
        sd = _rb(jnp.sqrt(_rb(_rb(v) + eps)))
        xn = (_rb(x - _rb(m)) * (1.0 / sd)).astype(bf16)
        xn_v[pl.ds(pl.multiple_of(b * R + 16 * q, 16), 16), :] = xn
        r = _rb(jnp.sum(xn.astype(f32) * wr, axis=-1, keepdims=True))
        for j in range(2):
            racc = jnp.where(lane == b * J + 2 * q + j, r[NSEG * j:NSEG * (j + 1), :], racc)
        return racc

    def stage(b, s, z=None):
        nat = pl.ds(pl.multiple_of(s * SEG + b * J, J), J)
        for g in range(G):
            zz = None if z is None else jnp.concatenate([z] * (J // 8), axis=0)
            st_v[g, s * PA:s * PA + J, :] = tie(x_v[nat, 128 * g:128 * (g + 1)].astype(f32), zz)

    def step(n, h, bu):
        ar, ai = ar8[:, 128 * n:128 * (n + 1)], ai8[:, 128 * n:128 * (n + 1)]
        return (ar * h[0] - ai * h[1] + bu[:, :128], ar * h[1] + ai * h[0] + bu[:, 128:])

    def in_proj(b, n, h):
        rows = pl.ds(pl.multiple_of(b * R, R), R)
        cols = slice(n * 256, (n + 1) * 256)
        bu = jax.lax.dot_general(xn_v[rows, :], b_v[cols, :], _NT, preferred_element_type=f32)
        bu_v[rows, cols] = bu
        for j in range(J):
            h = step(n, h, bu[NSEG * j:NSEG * (j + 1), :])
        t = pltpu.bitcast(bu[:, :128], jnp.int32)
        zs = [(t[8 * i:8 * i + 8] * t[8 * i:8 * i + 8]) & 2 for i in range(0, J, J // 4)]
        return h, zs

    def cprep(row, z):
        rows = pl.ds(pl.multiple_of(row, 16), 16)
        zz = jnp.concatenate([jnp.concatenate([z, z], axis=0)] * G, axis=1)
        cre = tie(craw_v[0, rows, :].astype(f32), zz)
        cim = craw_v[1, rows, :].astype(f32)
        xn_v[pl.ds(pl.multiple_of(L + row, 16), 16), :] = (cre * k_re - cim * k_im).astype(bf16)
        xn_v[pl.ds(pl.multiple_of(L + D + row, 16), 16), :] = (cre * (-k_im) - cim * k_re).astype(bf16)

    z = jnp.zeros((NSEG, 128), f32)
    hs = []
    for n in range(AHEAD):
        for cp in b_cp(n):
            cp.start()
    for s in range(NSEG):
        x_cp(0, s).wait()
    for s in range(NSEG):
        stage(0, s)
    racc = jnp.zeros((NSEG, SEG), f32)
    for q in range(R // 16):
        racc = norm_rows(0, q, racc)

    def phase_a(b, carry, with_c=False, first=False, last=False, second=False):
        hp, racc = carry
        hs = []
        if not last and not first:
            for s in range(NSEG):
                x_cp(b + 1, s).wait()

        for n in range(NA):
            if first and n in PLAN:
                waits, starts = PLAN[n]
                for kind, i in waits:
                    for cp in (b_cp(i) if kind == "b" else [x_cp(i, s) for s in range(NSEG)]):
                        cp.wait()
                for kind, i in starts:
                    for cp in (b_cp(i) if kind == "b" else [x_cp(i, s) for s in range(NSEG)]):
                        cp.start()
            if second and n == NA // 2:
                for cp in c_cps + f_cps:
                    cp.start()
            h, zs = in_proj(b, n, hp[n])
            hs.append(h)
            if not last and not first:
                if n < 2:
                    for i in range(4):
                        stage(b + 1, 4 * n + i, zs[i])
                else:
                    qs = range((n - 2) * 16 // 6, (n - 1) * 16 // 6)
                    for i, q in enumerate(qs):
                        racc = norm_rows(b + 1, q, racc, zs[i])
            if first and n == 4:
                for i in range(8):
                    stage(1, i, zs[i // 2])
            if first and n > 4:
                for i, q in enumerate(range((n - 5) * 16 // 3, (n - 4) * 16 // 3)):
                    racc = norm_rows(1, q, racc, zs[i % 4])
            if with_c:
                k = 2 * D // NB // NA
                for i in range(k // 16):
                    cprep(((b - NB // 2) * NA + n) * k + 16 * i, zs[2 * i + 1])
        return hs, racc

    hs, racc = phase_a(0, ([(z, z)] * NA, racc), first=True)
    hs = jax.lax.fori_loop(2, NB // 2, phase_a, phase_a(1, (hs, racc), second=True))
    for cp in c_cps:
        cp.wait()
    hs = jax.lax.fori_loop(
        NB // 2, NB - 1, lambda b, c: phase_a(b, c, True), hs)
    hs, racc = phase_a(NB - 1, hs, True, last=True)
    er = jnp.concatenate([h[0] for h in hs], axis=1)
    ei = jnp.concatenate([h[1] for h in hs], axis=1)
    pr, pi = ar8, ai8
    n = 1
    while n < SEG:
        pr, pi = pr * pr - pi * pi, 2.0 * pr * pi
        n *= 2
    srow = jax.lax.broadcasted_iota(jnp.int32, (NSEG, P), 0)
    hr = jnp.where(srow >= 1, pltpu.roll(er, 1, 0), 0.0)
    hi = jnp.where(srow >= 1, pltpu.roll(ei, 1, 0), 0.0)
    for sh in (1, 2, 4):
        tr = jnp.where(srow >= sh, pltpu.roll(hr, sh, 0), 0.0)
        ti = jnp.where(srow >= sh, pltpu.roll(hi, sh, 0), 0.0)
        hr, hi = hr + pr * tr - pi * ti, hi + pr * ti + pi * tr
        pr, pi = pr * pr - pi * pi, 2.0 * pr * pi

    tok = sub * SEG + lane
    r0 = jnp.max(racc)
    i0 = jnp.min(jnp.where(racc == r0, tok, L))
    rest = jnp.where(tok == i0, -jnp.inf, racc)
    r1 = jnp.max(rest)
    i1 = jnp.min(jnp.where((rest == r1) & (tok != i0), tok, L))
    i0 = jnp.clip(i0, 0, L - 1)
    i1 = jnp.clip(i1, 0, L - 1)
    p0 = (i0 % SEG) * NSEG + i0 // SEG
    p1 = (i1 % SEG) * NSEG + i1 // SEG
    r16 = jax.lax.broadcasted_iota(jnp.int32, (16, D), 0)

    def pick(p):
        g = xn_v[pl.ds(pl.multiple_of((p // 16) * 16, 16), 16), :].astype(f32)
        return jnp.sum(jnp.where(r16 == p % 16, g, 0.0), axis=0, keepdims=True)

    xs = jnp.where(r16 == 0, pick(p0), jnp.where(r16 == 1, pick(p1), 0.0)).astype(bf16)
    for cp in f_cps:
        cp.wait()
    g = _rb(jnp.dot(xs, wg_v[...], preferred_element_type=f32))
    u = _rb(jnp.dot(xs, wu_v[...], preferred_element_type=f32))
    g = _rb(g * jax.nn.sigmoid(g))
    y = _rb(jnp.dot((g * u).astype(bf16), wd_v[...], preferred_element_type=f32))
    rs = jnp.where(r16 == 0, r0, r1)
    y = _rb(y * _rb(jax.nn.sigmoid(rs)))
    y0 = y[0:1, :]
    y1 = y[1:2, :]
    rowt = jax.lax.broadcasted_iota(jnp.int32, (16, 128), 0)

    def states(b, n, h, z=None):
        base = pl.multiple_of(b * R, R)
        h = (tie(h[0], z), h[1])
        seq = []
        for j in range(J):
            h = step(n, h, bu_v[pl.ds(base + NSEG * j, NSEG), 256 * n:256 * (n + 1)])
            seq.append(jnp.concatenate(h, axis=1))
        return h, jnp.concatenate(seq, axis=0).astype(bf16)

    def unpermute(b, g, z=None):
        cg = slice(128 * g, 128 * (g + 1))
        zz = None if z is None else jnp.concatenate([z] * (J // 8), axis=0)
        for s in range(NSEG):
            nat = pl.ds(pl.multiple_of(s * SEG + b * J, J), J)
            o_v[nat, cg] = x_v[nat, cg].astype(f32) + tie(st_v[g, pl.ds(s, J, stride=PB), :], zz)

    def phase_b(b, carry, first=False, last=False):
        ys = None
        hs = list(carry)
        for n in range(G):
            if n == 0:
                hq = h_v[...]
            else:
                hs[n], hq = states(b, n, carry[n])
            cn = slice(128 * n, 128 * (n + 1))
            cw = jnp.concatenate([xn_v[L:L + D, cn], xn_v[L + D:, cn]], axis=1)
            y = jax.lax.dot_general(hq, cw, _NT, preferred_element_type=f32)
            ys = y if ys is None else ys + y
            zs = []
            for i in range(2):
                t = pltpu.bitcast(y[:8, 512 * i:512 * i + 128], jnp.int32)
                zs.append((t * t) & 2)
            if not first and n < 4:
                for i in range(2):
                    unpermute(b - 1, 2 * n + i, zs[i])
            if not last and n == G - 2:
                hs[0], hq0 = states(b + 1, 0, carry[0], zs[0])
                h_v[...] = hq0
        if not first:
            for s in range(NSEG):
                o_cp(b - 1, s).start()
        for g in range(G):
            cg = slice(128 * g, 128 * (g + 1))
            for q in range(R // 16):
                row = pl.multiple_of(b * R + 16 * q, 16)
                t = ys[16 * q:16 * (q + 1), cg]
                t = t + xn_v[pl.ds(row, 16), cg].astype(f32) * dsk1[:, cg]
                t = jnp.where(rowt == p0 - row, t + y0[:, cg], t)
                t = jnp.where(rowt == p1 - row, t + y1[:, cg], t)
                for j in range(2):
                    st_v[g, pl.ds(PB * (2 * q + j), 8), :] = t[8 * j:8 * (j + 1), :]
        return hs

    hs = [(hr[:, 128 * n:128 * (n + 1)], hi[:, 128 * n:128 * (n + 1)]) for n in range(G)]
    hs[0], hq = states(0, 0, hs[0])
    h_v[...] = hq
    hs = phase_b(0, hs, first=True)
    hs = jax.lax.fori_loop(1, NB - 1, phase_b, hs)
    phase_b(NB - 1, hs, last=True)
    for g in range(G):
        unpermute(NB - 1, g)
    for s in range(NSEG):
        o_cp(NB - 1, s).start()
    pltpu.make_async_copy(o_v, o_v, so.at[0]).wait()


@jax.jit
def pallas_parallel_sum__ssm_conv_s5__moe_arch_mod__prompt_kernel(
    A_x: jax.Array,
    A_Lambda_re: jax.Array,
    A_Lambda_im: jax.Array,
    A_B_re: jax.Array,
    A_B_im: jax.Array,
    A_C_re: jax.Array,
    A_C_im: jax.Array,
    A_log_dt: jax.Array,
    A_Dskip: jax.Array,
    B_x: jax.Array,
    B_w_r: jax.Array,
    B_w_gate: jax.Array,
    B_w_up: jax.Array,
    B_w_down: jax.Array,
):
    del B_x
    hbm = pl.BlockSpec(memory_space=pl.ANY)
    vec = pl.BlockSpec(memory_space=pltpu.VMEM)
    out = pl.pallas_call(
        _kernel,
        out_shape=jax.ShapeDtypeStruct((L, D), f32),
        in_specs=[hbm, vec, vec, hbm, hbm, hbm, hbm, vec, vec, vec, hbm, hbm, hbm],
        out_specs=hbm,
        scratch_shapes=[
            pltpu.VMEM((L, D), bf16),
            pltpu.VMEM((L + 2 * D, D), bf16),
            pltpu.VMEM((2 * P, D), bf16),
            pltpu.VMEM((2, D, P), bf16),
            pltpu.VMEM((L, 2 * P), f32),
            pltpu.VMEM((R, 256), bf16),
            pltpu.VMEM((L, D), f32),
            pltpu.VMEM((G, PB * J, 128), f32),
            pltpu.VMEM((D, F), bf16),
            pltpu.VMEM((D, F), bf16),
            pltpu.VMEM((F, D), bf16),
            pltpu.SemaphoreType.DMA((NB,)),
            pltpu.SemaphoreType.DMA((NA,)),
            pltpu.SemaphoreType.DMA((7,)),
            pltpu.SemaphoreType.DMA((1,)),
        ],
        compiler_params=pltpu.CompilerParams(vmem_limit_bytes=100 * 1024 * 1024),
    )(
        A_x.reshape(L, D),
        A_Lambda_re, A_Lambda_im,
        A_B_re, A_B_im, A_C_re, A_C_im,
        A_log_dt, A_Dskip, B_w_r,
        B_w_gate, B_w_up, B_w_down,
    )
    return out.reshape(1, L, D)
```

```python
import jax
import jax.numpy as jnp
import numpy as np
import jax.experimental.pallas as pl
import jax.experimental.pallas.tpu as pltpu

L = 2048
D = 1024
P = 1024
F = 3584
NSEG = 8
SEG = L // NSEG
J = 32
NB = SEG // J
R = NSEG * J
G = D // 128
NA = 8
PLAN = {0: ([('b', 0), ('b', 1)], [('b', 2), ('b', 3), ('x', 1), ('b', 4), ('b', 5)]), 2: ([('b', 2), ('b', 3)], [('b', 6), ('b', 7)]), 4: ([('b', 4), ('b', 5), ('x', 1)], [('x', 2)]), 6: ([('b', 6), ('b', 7)], [('x', 3), ('x', 4), ('x', 5), ('x', 6), ('x', 7)])}
AHEAD = 2
PA = J + 4
PB = 12

_NT = (((1,), (1,)), ((), ()))
f32 = jnp.float32
bf16 = jnp.bfloat16


def _rb(v):
    return v.astype(bf16).astype(f32)


def _kernel(x_hbm, lre_ref, lim_ref, bre_hbm, bim_hbm, cre_hbm, cim_hbm, ldt_ref,
            dsk_ref, wr_ref, wg_hbm, wu_hbm, wd_hbm, out_hbm,
            x_v, xn_v, b_v, craw_v, bu_v, h_v, o_v, st_v, wg_v, wu_v, wd_v,
            sx, sb, sw, so):
    def x_cp(b, s):
        rows = pl.ds(pl.multiple_of(s * SEG + b * J, J), J)
        return pltpu.make_async_copy(x_hbm.at[rows], x_v.at[rows], sx.at[b])

    def b_cp(n):
        return [pltpu.make_async_copy(src.at[pl.ds(n * 128, 128)],
                                      b_v.at[pl.ds(n * 256 + i * 128, 128)], sb.at[n])
                for i, src in enumerate((bre_hbm, bim_hbm))]

    def o_cp(b, s):
        rows = pl.ds(pl.multiple_of(s * SEG + b * J, J), J)
        return pltpu.make_async_copy(o_v.at[rows], out_hbm.at[rows], so.at[0])

    c_cps = [pltpu.make_async_copy(cre_hbm, craw_v.at[0], sw.at[2]),
             pltpu.make_async_copy(cim_hbm, craw_v.at[1], sw.at[3])]
    f_cps = [pltpu.make_async_copy(wg_hbm, wg_v, sw.at[4]),
             pltpu.make_async_copy(wu_hbm, wu_v, sw.at[5]),
             pltpu.make_async_copy(wd_hbm, wd_v, sw.at[6])]

    for b in range(1):
        for s in range(NSEG):
            x_cp(b, s).start()

    dt = _rb(jnp.exp(ldt_ref[...].astype(f32).reshape(1, D)))
    lre = lre_ref[...].astype(f32).reshape(1, D)
    lim = lim_ref[...].astype(f32).reshape(1, D)
    mag = jnp.exp(dt * lre)
    a_re = mag * jnp.cos(dt * lim)
    a_im = mag * jnp.sin(dt * lim)
    den = lre * lre + lim * lim
    k_re = 2.0 * ((a_re - 1.0) * lre + a_im * lim) / den
    k_im = 2.0 * (a_im * lre - (a_re - 1.0) * lim) / den
    ar8 = jnp.broadcast_to(a_re, (NSEG, P))
    ai8 = jnp.broadcast_to(a_im, (NSEG, P))
    wr = wr_ref[...].astype(f32).reshape(1, D)
    eps = f32(np.float32(np.asarray(1e-5, dtype=bf16)))

    dsk1 = dsk_ref[...].astype(f32).reshape(1, D) + 1.0
    lane = jax.lax.broadcasted_iota(jnp.int32, (NSEG, SEG), 1)
    sub = jax.lax.broadcasted_iota(jnp.int32, (NSEG, SEG), 0)

    def tie(v, z):
        return v if z is None else pltpu.bitcast(pltpu.bitcast(v, jnp.int32) | z, f32)

    def norm_rows(b, q, racc, z=None):
        x = jnp.concatenate([
            jnp.concatenate([tie(st_v[g, pl.ds(2 * q + j, NSEG, stride=PA), :], z if g == 0 else None) for g in range(G)], axis=1)
            for j in range(2)], axis=0)
        m = jnp.sum(x, axis=-1, keepdims=True) * (1.0 / D)
        c = x - m
        v = jnp.sum(c * c, axis=-1, keepdims=True) * (1.0 / D)
        sd = _rb(jnp.sqrt(_rb(_rb(v) + eps)))
        xn = (_rb(x - _rb(m)) * (1.0 / sd)).astype(bf16)
        xn_v[pl.ds(pl.multiple_of(b * R + 16 * q, 16), 16), :] = xn
        r = _rb(jnp.sum(xn.astype(f32) * wr, axis=-1, keepdims=True))
        for j in range(2):
            racc = jnp.where(lane == b * J + 2 * q + j, r[NSEG * j:NSEG * (j + 1), :], racc)
        return racc

    def stage(b, s, z=None):
        nat = pl.ds(pl.multiple_of(s * SEG + b * J, J), J)
        for g in range(G):
            zz = None if z is None else jnp.concatenate([z] * (J // 8), axis=0)
            st_v[g, s * PA:s * PA + J, :] = tie(x_v[nat, 128 * g:128 * (g + 1)].astype(f32), zz)

    def step(n, h, bu):
        ar, ai = ar8[:, 128 * n:128 * (n + 1)], ai8[:, 128 * n:128 * (n + 1)]
        return (ar * h[0] - ai * h[1] + bu[:, :128], ar * h[1] + ai * h[0] + bu[:, 128:])

    def in_proj(b, n, h):
        rows = pl.ds(pl.multiple_of(b * R, R), R)
        cols = slice(n * 256, (n + 1) * 256)
        bu = jax.lax.dot_general(xn_v[rows, :], b_v[cols, :], _NT, preferred_element_type=f32)
        bu_v[rows, cols] = bu
        for j in range(J):
            h = step(n, h, bu[NSEG * j:NSEG * (j + 1), :])
        t = pltpu.bitcast(bu[:, :128], jnp.int32)
        zs = [(t[8 * i:8 * i + 8] * t[8 * i:8 * i + 8]) & 2 for i in range(0, J, J // 4)]
        return h, zs

    def cprep(row, z):
        rows = pl.ds(pl.multiple_of(row, 16), 16)
        zz = jnp.concatenate([jnp.concatenate([z, z], axis=0)] * G, axis=1)
        cre = tie(craw_v[0, rows, :].astype(f32), zz)
        cim = craw_v[1, rows, :].astype(f32)
        xn_v[pl.ds(pl.multiple_of(L + row, 16), 16), :] = (cre * k_re - cim * k_im).astype(bf16)
        xn_v[pl.ds(pl.multiple_of(L + D + row, 16), 16), :] = (cre * (-k_im) - cim * k_re).astype(bf16)

    z = jnp.zeros((NSEG, 128), f32)
    hs = []
    for n in range(AHEAD):
        for cp in b_cp(n):
            cp.start()
    for s in range(NSEG):
        x_cp(0, s).wait()
    for s in range(NSEG):
        stage(0, s)
    racc = jnp.zeros((NSEG, SEG), f32)
    for q in range(R // 16):
        racc = norm_rows(0, q, racc)

    def phase_a(b, carry, with_c=False, first=False, last=False, second=False):
        hp, racc = carry
        hs = []
        if not last and not first:
            for s in range(NSEG):
                x_cp(b + 1, s).wait()

        for n in range(NA):
            if first and n in PLAN:
                waits, starts = PLAN[n]
                for kind, i in waits:
                    for cp in (b_cp(i) if kind == "b" else [x_cp(i, s) for s in range(NSEG)]):
                        cp.wait()
                for kind, i in starts:
                    for cp in (b_cp(i) if kind == "b" else [x_cp(i, s) for s in range(NSEG)]):
                        cp.start()
            if second and n == NA // 2:
                for cp in c_cps + f_cps:
                    cp.start()
            h, zs = in_proj(b, n, hp[n])
            hs.append(h)
            if not last and not first:
                if n < 2:
                    for i in range(4):
                        stage(b + 1, 4 * n + i, zs[i])
                else:
                    qs = range((n - 2) * 16 // 6, (n - 1) * 16 // 6)
                    for i, q in enumerate(qs):
                        racc = norm_rows(b + 1, q, racc, zs[i])
            if first and n == 4:
                for i in range(8):
                    stage(1, i, zs[i // 2])
            if first and n > 4:
                for i, q in enumerate(range((n - 5) * 16 // 3, (n - 4) * 16 // 3)):
                    racc = norm_rows(1, q, racc, zs[i % 4])
            if with_c:
                k = 2 * D // NB // NA
                for i in range(k // 16):
                    cprep(((b - NB // 2) * NA + n) * k + 16 * i, zs[2 * i + 1])
        return hs, racc

    hs, racc = phase_a(0, ([(z, z)] * NA, racc), first=True)
    hs = jax.lax.fori_loop(2, NB // 2, phase_a, phase_a(1, (hs, racc), second=True))
    for cp in c_cps:
        cp.wait()
    hs = jax.lax.fori_loop(
        NB // 2, NB - 1, lambda b, c: phase_a(b, c, True), hs)
    hs, racc = phase_a(NB - 1, hs, True, last=True)
    er = jnp.concatenate([h[0] for h in hs], axis=1)
    ei = jnp.concatenate([h[1] for h in hs], axis=1)
    pr, pi = ar8, ai8
    n = 1
    while n < SEG:
        pr, pi = pr * pr - pi * pi, 2.0 * pr * pi
        n *= 2
    srow = jax.lax.broadcasted_iota(jnp.int32, (NSEG, P), 0)
    hr = jnp.where(srow >= 1, pltpu.roll(er, 1, 0), 0.0)
    hi = jnp.where(srow >= 1, pltpu.roll(ei, 1, 0), 0.0)
    for sh in (1, 2, 4):
        tr = jnp.where(srow >= sh, pltpu.roll(hr, sh, 0), 0.0)
        ti = jnp.where(srow >= sh, pltpu.roll(hi, sh, 0), 0.0)
        hr, hi = hr + pr * tr - pi * ti, hi + pr * ti + pi * tr
        pr, pi = pr * pr - pi * pi, 2.0 * pr * pi

    rowt = jax.lax.broadcasted_iota(jnp.int32, (8, D), 0)

    def states(b, n, h, z=None):
        base = pl.multiple_of(b * R, R)
        h = (tie(h[0], z), h[1])
        seq = []
        for j in range(J):
            h = step(n, h, bu_v[pl.ds(base + NSEG * j, NSEG), 256 * n:256 * (n + 1)])
            seq.append(jnp.concatenate(h, axis=1))
        return h, jnp.concatenate(seq, axis=0).astype(bf16)

    def unpermute(b, g, z=None):
        cg = slice(128 * g, 128 * (g + 1))
        zz = None if z is None else jnp.concatenate([z] * (J // 8), axis=0)
        for s in range(NSEG):
            nat = pl.ds(pl.multiple_of(s * SEG + b * J, J), J)
            o_v[nat, cg] = x_v[nat, cg].astype(f32) + tie(st_v[g, pl.ds(s, J, stride=PB), :], zz)

    def phase_b(b, carry, first=False, last=False):
        ys = None
        hs = list(carry)
        for n in range(G):
            if n == 0:
                hq = h_v[...]
            else:
                hs[n], hq = states(b, n, carry[n])
            cn = slice(128 * n, 128 * (n + 1))
            cw = jnp.concatenate([xn_v[L:L + D, cn], xn_v[L + D:, cn]], axis=1)
            y = jax.lax.dot_general(hq, cw, _NT, preferred_element_type=f32)
            ys = y if ys is None else ys + y
            zs = []
            for i in range(2):
                t = pltpu.bitcast(y[:8, 512 * i:512 * i + 128], jnp.int32)
                zs.append((t * t) & 2)
            if not first and n < 4:
                for i in range(2):
                    unpermute(b - 1, 2 * n + i, zs[i])
            if not last and n == G - 2:
                hs[0], hq0 = states(b + 1, 0, carry[0], zs[0])
                h_v[...] = hq0
        if not first:
            release(b - 1)
        for g in range(G):
            cg = slice(128 * g, 128 * (g + 1))
            for q in range(R // 16):
                row = pl.multiple_of(b * R + 16 * q, 16)
                t = ys[16 * q:16 * (q + 1), cg]
                t = t + xn_v[pl.ds(row, 16), cg].astype(f32) * dsk1[:, cg]
                for j in range(2):
                    st_v[g, pl.ds(PB * (2 * q + j), 8), :] = t[8 * j:8 * (j + 1), :]
        return hs

    def release(b):
        for tok_i, upd in ((i0, y0), (i1, y1)):
            row0 = jnp.where((tok_i % SEG) // J == b, (tok_i // 8) * 8, L)
            grp = pl.ds(pl.multiple_of(row0, 8), 8)
            o_v[grp, :] += jnp.where(rowt == tok_i % 8, upd, 0.0)
        for s in range(NSEG):
            o_cp(b, s).start()

    o_v[L:, :] = jnp.zeros((8, D), f32)
    hs = [(hr[:, 128 * n:128 * (n + 1)], hi[:, 128 * n:128 * (n + 1)]) for n in range(G)]
    hs[0], hq = states(0, 0, hs[0])
    h_v[...] = hq
    hs = phase_b(0, hs, first=True)
    tok = sub * SEG + lane
    r0 = jnp.max(racc)
    i0 = jnp.min(jnp.where(racc == r0, tok, L))
    rest = jnp.where(tok == i0, -jnp.inf, racc)
    r1 = jnp.max(rest)
    i1 = jnp.min(jnp.where((rest == r1) & (tok != i0), tok, L))
    i0 = jnp.clip(i0, 0, L - 1)
    i1 = jnp.clip(i1, 0, L - 1)
    p0 = (i0 % SEG) * NSEG + i0 // SEG
    p1 = (i1 % SEG) * NSEG + i1 // SEG
    r16 = jax.lax.broadcasted_iota(jnp.int32, (16, D), 0)

    def pick(p):
        g = xn_v[pl.ds(pl.multiple_of((p // 16) * 16, 16), 16), :].astype(f32)
        return jnp.sum(jnp.where(r16 == p % 16, g, 0.0), axis=0, keepdims=True)

    xs = jnp.where(r16 == 0, pick(p0), jnp.where(r16 == 1, pick(p1), 0.0)).astype(bf16)
    for cp in f_cps:
        cp.wait()
    g = _rb(jnp.dot(xs, wg_v[...], preferred_element_type=f32))
    u = _rb(jnp.dot(xs, wu_v[...], preferred_element_type=f32))
    g = _rb(g * jax.nn.sigmoid(g))
    y = _rb(jnp.dot((g * u).astype(bf16), wd_v[...], preferred_element_type=f32))
    rs = jnp.where(r16 == 0, r0, r1)
    y = _rb(y * _rb(jax.nn.sigmoid(rs)))
    y0 = y[0:1, :]
    y1 = y[1:2, :]
    hs = jax.lax.fori_loop(1, NB - 1, phase_b, hs)
    phase_b(NB - 1, hs, last=True)
    for g in range(G):
        unpermute(NB - 1, g)
    release(NB - 1)
    pltpu.make_async_copy(o_v.at[pl.ds(0, L)], out_hbm, so.at[0]).wait()


@jax.jit
def pallas_parallel_sum__ssm_conv_s5__moe_arch_mod__prompt_kernel(
    A_x: jax.Array,
    A_Lambda_re: jax.Array,
    A_Lambda_im: jax.Array,
    A_B_re: jax.Array,
    A_B_im: jax.Array,
    A_C_re: jax.Array,
    A_C_im: jax.Array,
    A_log_dt: jax.Array,
    A_Dskip: jax.Array,
    B_x: jax.Array,
    B_w_r: jax.Array,
    B_w_gate: jax.Array,
    B_w_up: jax.Array,
    B_w_down: jax.Array,
):
    del B_x
    hbm = pl.BlockSpec(memory_space=pl.ANY)
    vec = pl.BlockSpec(memory_space=pltpu.VMEM)
    out = pl.pallas_call(
        _kernel,
        out_shape=jax.ShapeDtypeStruct((L, D), f32),
        in_specs=[hbm, vec, vec, hbm, hbm, hbm, hbm, vec, vec, vec, hbm, hbm, hbm],
        out_specs=hbm,
        scratch_shapes=[
            pltpu.VMEM((L, D), bf16),
            pltpu.VMEM((L + 2 * D, D), bf16),
            pltpu.VMEM((2 * P, D), bf16),
            pltpu.VMEM((2, D, P), bf16),
            pltpu.VMEM((L, 2 * P), f32),
            pltpu.VMEM((R, 256), bf16),
            pltpu.VMEM((L + 8, D), f32),
            pltpu.VMEM((G, PB * J, 128), f32),
            pltpu.VMEM((D, F), bf16),
            pltpu.VMEM((D, F), bf16),
            pltpu.VMEM((F, D), bf16),
            pltpu.SemaphoreType.DMA((NB,)),
            pltpu.SemaphoreType.DMA((NA,)),
            pltpu.SemaphoreType.DMA((7,)),
            pltpu.SemaphoreType.DMA((1,)),
        ],
        compiler_params=pltpu.CompilerParams(vmem_limit_bytes=100 * 1024 * 1024),
    )(
        A_x.reshape(L, D),
        A_Lambda_re, A_Lambda_im,
        A_B_re, A_B_im, A_C_re, A_C_im,
        A_log_dt, A_Dskip, B_w_r,
        B_w_gate, B_w_up, B_w_down,
    )
    return out.reshape(1, L, D)
```

```python
import jax
import jax.numpy as jnp
import numpy as np
import jax.experimental.pallas as pl
import jax.experimental.pallas.tpu as pltpu

L = 2048
D = 1024
P = 1024
F = 3584
NSEG = 8
SEG = L // NSEG
J = 32
NB = SEG // J
R = NSEG * J
G = D // 128
NA = 8
PLAN = {0: ([('b', 0), ('b', 1)], [('b', 2), ('b', 3), ('x', 1), ('b', 4), ('b', 5)]), 2: ([('b', 2), ('b', 3)], [('b', 6), ('b', 7)]), 4: ([('b', 4), ('b', 5), ('x', 1)], [('x', 2)]), 6: ([('b', 6), ('b', 7)], [('x', 3), ('x', 4), ('x', 5), ('x', 6), ('x', 7)])}
AHEAD = 2
PA = J + 4
PB = 12

_NT = (((1,), (1,)), ((), ()))
f32 = jnp.float32
bf16 = jnp.bfloat16


def _rb(v):
    return v.astype(bf16).astype(f32)


def _kernel(x_hbm, lre_ref, lim_ref, bre_hbm, bim_hbm, cre_hbm, cim_hbm, ldt_ref,
            dsk_ref, wr_ref, wg_hbm, wu_hbm, wd_hbm, out_hbm,
            x_v, xn_v, b_v, craw_v, bu_v, h_v, o_v, st_v, wg_v, wu_v, wd_v,
            sx, sb, sw, so):
    def x_cp(b, s):
        rows = pl.ds(pl.multiple_of(s * SEG + b * J, J), J)
        return pltpu.make_async_copy(x_hbm.at[rows], x_v.at[rows], sx.at[b])

    def b_cp(n):
        return [pltpu.make_async_copy(src.at[pl.ds(n * 128, 128)],
                                      b_v.at[pl.ds(n * 256 + i * 128, 128)], sb.at[n])
                for i, src in enumerate((bre_hbm, bim_hbm))]

    def o_cp(b, s):
        rows = pl.ds(pl.multiple_of(s * SEG + b * J, J), J)
        return pltpu.make_async_copy(o_v.at[rows], out_hbm.at[rows], so.at[0])

    c_cps = [pltpu.make_async_copy(cre_hbm, craw_v.at[0], sw.at[2]),
             pltpu.make_async_copy(cim_hbm, craw_v.at[1], sw.at[3])]
    f_cps = [pltpu.make_async_copy(wg_hbm, wg_v, sw.at[4]),
             pltpu.make_async_copy(wu_hbm, wu_v, sw.at[5]),
             pltpu.make_async_copy(wd_hbm, wd_v, sw.at[6])]

    for b in range(1):
        for s in range(NSEG):
            x_cp(b, s).start()

    dt = _rb(jnp.exp(ldt_ref[...].astype(f32).reshape(1, D)))
    lre = lre_ref[...].astype(f32).reshape(1, D)
    lim = lim_ref[...].astype(f32).reshape(1, D)
    mag = jnp.exp(dt * lre)
    a_re = mag * jnp.cos(dt * lim)
    a_im = mag * jnp.sin(dt * lim)
    den = lre * lre + lim * lim
    k_re = 2.0 * ((a_re - 1.0) * lre + a_im * lim) / den
    k_im = 2.0 * (a_im * lre - (a_re - 1.0) * lim) / den
    ar8 = jnp.broadcast_to(a_re, (NSEG, P))
    ai8 = jnp.broadcast_to(a_im, (NSEG, P))
    wr = wr_ref[...].astype(f32).reshape(1, D)
    eps = f32(np.float32(np.asarray(1e-5, dtype=bf16)))

    dsk1 = dsk_ref[...].astype(f32).reshape(1, D) + 1.0
    lane = jax.lax.broadcasted_iota(jnp.int32, (NSEG, SEG), 1)
    sub = jax.lax.broadcasted_iota(jnp.int32, (NSEG, SEG), 0)

    def tie(v, z):
        return v if z is None else pltpu.bitcast(pltpu.bitcast(v, jnp.int32) | z, f32)

    def norm_rows(b, q, racc, z=None):
        x = jnp.concatenate([
            jnp.concatenate([tie(st_v[g, pl.ds(2 * q + j, NSEG, stride=PA), :], z if g == 0 else None) for g in range(G)], axis=1)
            for j in range(2)], axis=0)
        m = jnp.sum(x, axis=-1, keepdims=True) * (1.0 / D)
        c = x - m
        v = jnp.sum(c * c, axis=-1, keepdims=True) * (1.0 / D)
        sd = _rb(jnp.sqrt(_rb(_rb(v) + eps)))
        xn = (_rb(x - _rb(m)) * (1.0 / sd)).astype(bf16)
        xn_v[pl.ds(pl.multiple_of(b * R + 16 * q, 16), 16), :] = xn
        r = _rb(jnp.sum(xn.astype(f32) * wr, axis=-1, keepdims=True))
        for j in range(2):
            racc = jnp.where(lane == b * J + 2 * q + j, r[NSEG * j:NSEG * (j + 1), :], racc)
        return racc

    def stage(b, s, z=None):
        nat = pl.ds(pl.multiple_of(s * SEG + b * J, J), J)
        for g in range(G):
            zz = None if z is None else jnp.concatenate([z] * (J // 8), axis=0)
            st_v[g, s * PA:s * PA + J, :] = tie(x_v[nat, 128 * g:128 * (g + 1)].astype(f32), zz)

    def step(n, h, bu):
        ar, ai = ar8[:, 128 * n:128 * (n + 1)], ai8[:, 128 * n:128 * (n + 1)]
        return (ar * h[0] - ai * h[1] + bu[:, :128], ar * h[1] + ai * h[0] + bu[:, 128:])

    def in_proj(b, n, h):
        rows = pl.ds(pl.multiple_of(b * R, R), R)
        cols = slice(n * 256, (n + 1) * 256)
        bu = jax.lax.dot_general(xn_v[rows, :], b_v[cols, :], _NT, preferred_element_type=f32)
        bu_v[rows, cols] = bu
        for j in range(J):
            h = step(n, h, bu[NSEG * j:NSEG * (j + 1), :])
        t = pltpu.bitcast(bu[:, :128], jnp.int32)
        zs = [(t[8 * i:8 * i + 8] * t[8 * i:8 * i + 8]) & 2 for i in range(0, J, J // 4)]
        return h, zs

    def cprep(row, z):
        rows = pl.ds(pl.multiple_of(row, 16), 16)
        zz = jnp.concatenate([jnp.concatenate([z, z], axis=0)] * G, axis=1)
        cre = tie(craw_v[0, rows, :].astype(f32), zz)
        cim = craw_v[1, rows, :].astype(f32)
        xn_v[pl.ds(pl.multiple_of(L + row, 16), 16), :] = (cre * k_re - cim * k_im).astype(bf16)
        xn_v[pl.ds(pl.multiple_of(L + D + row, 16), 16), :] = (cre * (-k_im) - cim * k_re).astype(bf16)

    z = jnp.zeros((NSEG, 128), f32)
    hs = []
    for n in range(AHEAD):
        for cp in b_cp(n):
            cp.start()
    for s in range(NSEG):
        x_cp(0, s).wait()
    for s in range(NSEG):
        stage(0, s)
    racc = jnp.zeros((NSEG, SEG), f32)
    for q in range(R // 16):
        racc = norm_rows(0, q, racc)

    def phase_a(b, carry, with_c=False, first=False, last=False, second=False):
        hp, racc = carry
        hs = []
        if not last and not first:
            for s in range(NSEG):
                x_cp(b + 1, s).wait()

        for n in range(NA):
            if first and n in PLAN:
                waits, starts = PLAN[n]
                for kind, i in waits:
                    for cp in (b_cp(i) if kind == "b" else [x_cp(i, s) for s in range(NSEG)]):
                        cp.wait()
                for kind, i in starts:
                    for cp in (b_cp(i) if kind == "b" else [x_cp(i, s) for s in range(NSEG)]):
                        cp.start()
            if second and n == NA // 2:
                for cp in c_cps:
                    cp.start()
            h, zs = in_proj(b, n, hp[n])
            hs.append(h)
            if not last and not first:
                if n < 2:
                    for i in range(4):
                        stage(b + 1, 4 * n + i, zs[i])
                else:
                    qs = range((n - 2) * 16 // 6, (n - 1) * 16 // 6)
                    for i, q in enumerate(qs):
                        racc = norm_rows(b + 1, q, racc, zs[i])
            if first and n == 4:
                for i in range(8):
                    stage(1, i, zs[i // 2])
            if first and n > 4:
                for i, q in enumerate(range((n - 5) * 16 // 3, (n - 4) * 16 // 3)):
                    racc = norm_rows(1, q, racc, zs[i % 4])
            if with_c:
                k = 2 * D // NB // NA
                for i in range(k // 16):
                    cprep(((b - NB // 2) * NA + n) * k + 16 * i, zs[2 * i + 1])
        return hs, racc

    hs, racc = phase_a(0, ([(z, z)] * NA, racc), first=True)
    hs = phase_a(1, (hs, racc), second=True)
    for cp in f_cps:
        cp.start()
    hs = jax.lax.fori_loop(2, NB // 2, phase_a, hs)
    for cp in c_cps:
        cp.wait()
    hs = jax.lax.fori_loop(
        NB // 2, NB - 1, lambda b, c: phase_a(b, c, True), hs)
    hs, racc = phase_a(NB - 1, hs, True, last=True)
    er = jnp.concatenate([h[0] for h in hs], axis=1)
    ei = jnp.concatenate([h[1] for h in hs], axis=1)
    pr, pi = ar8, ai8
    n = 1
    while n < SEG:
        pr, pi = pr * pr - pi * pi, 2.0 * pr * pi
        n *= 2
    srow = jax.lax.broadcasted_iota(jnp.int32, (NSEG, P), 0)
    hr = jnp.where(srow >= 1, pltpu.roll(er, 1, 0), 0.0)
    hi = jnp.where(srow >= 1, pltpu.roll(ei, 1, 0), 0.0)
    for sh in (1, 2, 4):
        tr = jnp.where(srow >= sh, pltpu.roll(hr, sh, 0), 0.0)
        ti = jnp.where(srow >= sh, pltpu.roll(hi, sh, 0), 0.0)
        hr, hi = hr + pr * tr - pi * ti, hi + pr * ti + pi * tr
        pr, pi = pr * pr - pi * pi, 2.0 * pr * pi

    rowt = jax.lax.broadcasted_iota(jnp.int32, (8, D), 0)

    def states(b, n, h, z=None):
        base = pl.multiple_of(b * R, R)
        h = (tie(h[0], z), h[1])
        seq = []
        for j in range(J):
            h = step(n, h, bu_v[pl.ds(base + NSEG * j, NSEG), 256 * n:256 * (n + 1)])
            seq.append(jnp.concatenate(h, axis=1))
        return h, jnp.concatenate(seq, axis=0).astype(bf16)

    def unpermute(b, g, z=None):
        cg = slice(128 * g, 128 * (g + 1))
        zz = None if z is None else jnp.concatenate([z] * (J // 8), axis=0)
        for s in range(NSEG):
            nat = pl.ds(pl.multiple_of(s * SEG + b * J, J), J)
            o_v[nat, cg] = x_v[nat, cg].astype(f32) + tie(st_v[g, pl.ds(s, J, stride=PB), :], zz)

    def phase_b(b, carry, first=False, last=False):
        ys = None
        hs = list(carry)
        for n in range(G):
            if n == 0:
                hq = h_v[...]
            else:
                hs[n], hq = states(b, n, carry[n])
            cn = slice(128 * n, 128 * (n + 1))
            cw = jnp.concatenate([xn_v[L:L + D, cn], xn_v[L + D:, cn]], axis=1)
            y = jax.lax.dot_general(hq, cw, _NT, preferred_element_type=f32)
            ys = y if ys is None else ys + y
            zs = []
            for i in range(2):
                t = pltpu.bitcast(y[:8, 512 * i:512 * i + 128], jnp.int32)
                zs.append((t * t) & 2)
            if not first and n < 4:
                for i in range(2):
                    unpermute(b - 1, 2 * n + i, zs[i])
            if not last and n == G - 2:
                hs[0], hq0 = states(b + 1, 0, carry[0], zs[0])
                h_v[...] = hq0
        if first:
            hs.append(zs[0])
        if not first:
            release(b - 1)
        for g in range(G):
            cg = slice(128 * g, 128 * (g + 1))
            for q in range(R // 16):
                row = pl.multiple_of(b * R + 16 * q, 16)
                t = ys[16 * q:16 * (q + 1), cg]
                t = t + xn_v[pl.ds(row, 16), cg].astype(f32) * dsk1[:, cg]
                for j in range(2):
                    st_v[g, pl.ds(PB * (2 * q + j), 8), :] = t[8 * j:8 * (j + 1), :]
        return hs

    def release(b):
        for tok_i, upd in ((i0, y0), (i1, y1)):
            row0 = jnp.where((tok_i % SEG) // J == b, (tok_i // 8) * 8, L)
            grp = pl.ds(pl.multiple_of(row0, 8), 8)
            o_v[grp, :] += jnp.where(rowt == tok_i % 8, upd, 0.0)
        for s in range(NSEG):
            o_cp(b, s).start()

    o_v[L:, :] = jnp.zeros((8, D), f32)
    hs = [(hr[:, 128 * n:128 * (n + 1)], hi[:, 128 * n:128 * (n + 1)]) for n in range(G)]
    hs[0], hq = states(0, 0, hs[0])
    h_v[...] = hq
    hs = phase_b(0, hs, first=True)
    z0 = hs.pop()
    racc = tie(racc, jnp.concatenate([z0, z0], axis=1))
    tok = sub * SEG + lane
    r0 = jnp.max(racc)
    i0 = jnp.min(jnp.where(racc == r0, tok, L))
    rest = jnp.where(tok == i0, -jnp.inf, racc)
    r1 = jnp.max(rest)
    i1 = jnp.min(jnp.where((rest == r1) & (tok != i0), tok, L))
    i0 = jnp.clip(i0, 0, L - 1)
    i1 = jnp.clip(i1, 0, L - 1)
    p0 = (i0 % SEG) * NSEG + i0 // SEG
    p1 = (i1 % SEG) * NSEG + i1 // SEG
    r16 = jax.lax.broadcasted_iota(jnp.int32, (16, D), 0)

    def pick(p):
        g = xn_v[pl.ds(pl.multiple_of((p // 16) * 16, 16), 16), :].astype(f32)
        return jnp.sum(jnp.where(r16 == p % 16, g, 0.0), axis=0, keepdims=True)

    xs = jnp.where(r16 == 0, pick(p0), jnp.where(r16 == 1, pick(p1), 0.0)).astype(bf16)
    for cp in f_cps:
        cp.wait()
    g = _rb(jnp.dot(xs, wg_v[...], preferred_element_type=f32))
    u = _rb(jnp.dot(xs, wu_v[...], preferred_element_type=f32))
    g = _rb(g * jax.nn.sigmoid(g))
    y = _rb(jnp.dot((g * u).astype(bf16), wd_v[...], preferred_element_type=f32))
    rs = jnp.where(r16 == 0, r0, r1)
    y = _rb(y * _rb(jax.nn.sigmoid(rs)))
    y0 = y[0:1, :]
    y1 = y[1:2, :]
    hs = jax.lax.fori_loop(1, NB - 1, phase_b, hs)
    phase_b(NB - 1, hs, last=True)
    for g in range(G):
        unpermute(NB - 1, g)
    release(NB - 1)
    pltpu.make_async_copy(o_v.at[pl.ds(0, L)], out_hbm, so.at[0]).wait()


@jax.jit
def pallas_parallel_sum__ssm_conv_s5__moe_arch_mod__prompt_kernel(
    A_x: jax.Array,
    A_Lambda_re: jax.Array,
    A_Lambda_im: jax.Array,
    A_B_re: jax.Array,
    A_B_im: jax.Array,
    A_C_re: jax.Array,
    A_C_im: jax.Array,
    A_log_dt: jax.Array,
    A_Dskip: jax.Array,
    B_x: jax.Array,
    B_w_r: jax.Array,
    B_w_gate: jax.Array,
    B_w_up: jax.Array,
    B_w_down: jax.Array,
):
    del B_x
    hbm = pl.BlockSpec(memory_space=pl.ANY)
    vec = pl.BlockSpec(memory_space=pltpu.VMEM)
    out = pl.pallas_call(
        _kernel,
        out_shape=jax.ShapeDtypeStruct((L, D), f32),
        in_specs=[hbm, vec, vec, hbm, hbm, hbm, hbm, vec, vec, vec, hbm, hbm, hbm],
        out_specs=hbm,
        scratch_shapes=[
            pltpu.VMEM((L, D), bf16),
            pltpu.VMEM((L + 2 * D, D), bf16),
            pltpu.VMEM((2 * P, D), bf16),
            pltpu.VMEM((2, D, P), bf16),
            pltpu.VMEM((L, 2 * P), f32),
            pltpu.VMEM((R, 256), bf16),
            pltpu.VMEM((L + 8, D), f32),
            pltpu.VMEM((G, PB * J, 128), f32),
            pltpu.VMEM((D, F), bf16),
            pltpu.VMEM((D, F), bf16),
            pltpu.VMEM((F, D), bf16),
            pltpu.SemaphoreType.DMA((NB,)),
            pltpu.SemaphoreType.DMA((NA,)),
            pltpu.SemaphoreType.DMA((7,)),
            pltpu.SemaphoreType.DMA((1,)),
        ],
        compiler_params=pltpu.CompilerParams(vmem_limit_bytes=100 * 1024 * 1024),
    )(
        A_x.reshape(L, D),
        A_Lambda_re, A_Lambda_im,
        A_B_re, A_B_im, A_C_re, A_C_im,
        A_log_dt, A_Dskip, B_w_r,
        B_w_gate, B_w_up, B_w_down,
    )
    return out.reshape(1, L, D)
```
